```python
import os as _os
_os.environ.setdefault('JAX_PLATFORMS', 'cpu')
import jax
import jax.numpy as jnp

def _softmax(x, axis=-1):
    return jax.nn.softmax(x, axis=axis)

def _gelu(x):
    return jax.nn.gelu(x, approximate=True)

def _silu(x):
    return jax.nn.silu(x)

def _sigmoid(x):
    return jax.nn.sigmoid(x)

def _layernorm(x, axis=-1, eps=1e-05):
    m = jnp.mean(x, axis=axis, keepdims=True)
    v = jnp.var(x, axis=axis, keepdims=True)
    return (x - m) / jnp.sqrt(v + eps)

def _scatter_add(tgt, idx, src, axis=0):
    return tgt.at[idx].add(src)

def _segment_sum(src, seg, n):
    return jax.ops.segment_sum(src, seg, n)

class _Rng:

    def __init__(self, key):
        self._k = key

    def _next(self):
        self._k, sub = jax.random.split(self._k)
        return sub

    def normal(self, shape):
        return jax.random.normal(self._next(), shape, dtype=jnp.bfloat16)

    def randint(self, lo, hi, shape):
        return jax.random.randint(self._next(), shape, lo, hi, dtype=jnp.int32)

    def uniform(self, shape, lo=0.0, hi=1.0):
        return jax.random.uniform(self._next(), shape, jnp.bfloat16, lo, hi)

    def permutation(self, n):
        return jax.random.permutation(self._next(), n)
kernel_name = 'adaLN_cond__mha_block__dense_activation_squared_relu__prompt'

def setup_inputs():
    _rng = _Rng(jax.random.key(int.from_bytes(__import__("os").urandom(4), "little")))
    _w = lambda a: (lambda t: t.astype(jnp.bfloat16) if jnp.issubdtype(t.dtype, jnp.floating) else t)(jnp.asarray(a))

    def _A_setup():
        B, S, D, H = (1, 2048, 512, 32)
        return {'x': _w((lambda *s: _rng.normal(s) * 0.05)(B, S, D)), 'wqkv': _w((lambda *s: _rng.normal(s) * 0.1)(D, 3 * D)), 'wo': _w((lambda *s: _rng.normal(s) * 0.05)(D, D))}
    _A_in = _A_setup()

    def _B_setup():
        B, S, D, F = (1, 2048, 512, 1792)
        return {'x': _w((lambda *s: _rng.normal(s) * 0.05)(B, S, D)), 'w1': _w((lambda *s: _rng.normal(s) * 0.05)(D, F)), 'b1': _w((lambda *s: _rng.normal(s) * 0.05)(F)), 'w2': _w((lambda *s: _rng.normal(s) * 0.05)(F, D)), 'b2': _w((lambda *s: _rng.normal(s) * 0.05)(D))}
    _B_in = _B_setup()
    return {'A_x': _A_in['x'], 'A_wqkv': _A_in['wqkv'], 'A_wo': _A_in['wo'], 'B_x': _B_in['x'], 'B_w1': _B_in['w1'], 'B_b1': _B_in['b1'], 'B_w2': _B_in['w2'], 'B_b2': _B_in['b2'], 'c': _w((lambda *s: _rng.normal(s) * 0.05)(1, 512) * 8.0), 'w_mod': _w((lambda *s: _rng.normal(s) * 0.05)(512, 6 * 512) * 512 ** (-0.5) * 8.0)}

def reference(A_x, A_wqkv, A_wo, B_x, B_w1, B_b1, B_w2, B_b2, c, w_mod):

    def _A_ref(x, wqkv, wo):
        B, S, D = x.shape
        H = 32
        Dh = D // H
        qkv = (lambda x, *d: x.transpose(*d))((x @ wqkv).reshape(B, S, 3, H, Dh), 2, 0, 3, 1, 4)
        q, k, v = (qkv[0], qkv[1], qkv[2])
        scores = jnp.einsum('bhqd,bhkd->bhqk', q, k) * Dh ** (-0.5)
        p = _softmax(scores, axis=-1)
        o = jnp.einsum('bhqk,bhkd->bhqd', p, v)
        return (lambda x, *d: x.transpose(*d))(o, 0, 2, 1, 3).reshape(B, S, D) @ wo

    def _B_ref(x, w1, b1, w2, b2):
        h = jnp.einsum('bsd,df->bsf', x, w1) + b1
        zero = jnp.zeros_like(h)
        r = jnp.where(h > zero, h, zero)
        h = r * r
        out = jnp.einsum('bsf,fd->bsd', h, w2) + b2
        return out
    x = A_x
    mod = (_silu(c) @ w_mod).reshape(c.shape[0], 6, 1, -1)
    sa, ca, ga, sb, cb, gb = (mod[:, 0].copy(), mod[:, 1].copy(), mod[:, 2].copy(), mod[:, 3].copy(), mod[:, 4].copy(), mod[:, 5].copy())
    h = _layernorm(x, axis=-1) * (1 + ca) + sa
    x = x + ga * _A_ref(h, A_wqkv, A_wo)
    h = _layernorm(x, axis=-1) * (1 + cb) + sb
    x = x + gb * _B_ref(h, B_w1, B_b1, B_w2, B_b2)
    return x
```

```python
import functools
import numpy as np
import jax, jax.numpy as jnp
from jax import lax
from jax.experimental import pallas as pl
from jax.experimental.pallas import tpu as pltpu

S, D, H, DH, F = 2048, 512, 32, 16, 1792
QSCALE = 0.25 * 1.4426950408889634
EPS = 1e-5
NT = (((1,), (1,)), ((), ()))
TN = (((0,), (0,)), ((), ()))
f32 = jnp.float32
bf16 = jnp.bfloat16


def _ln(x):
    m = jnp.mean(x, axis=-1, keepdims=True)
    d = x - m
    v = jnp.mean(d * d, axis=-1, keepdims=True)
    return d * lax.rsqrt(v + EPS)


def make_kernel(bq=512, kc=128, r1=512, r2=256):
    nq = S // bq
    nc = S // kc

    def kernel(x_ref, xq_ref, wqkv_ref, wo_ref, w1_ref, b1_ref, w2_ref, b2_ref, c_ref, wmod_ref,
               o_ref, mod_s, q_s, k_s, vT_s, sA, sB, oT_s):
        step_id = pl.program_id(0)

        @pl.when(step_id == 0)
        def _():
            c = c_ref[...].astype(f32)
            sc = c * jax.nn.sigmoid(c)
            sc = jnp.broadcast_to(sc, (16, D)).astype(bf16)
            mod = jnp.dot(sc, wmod_ref[...], preferred_element_type=f32)
            mod_s[...] = mod[0:8]
            wvT = wqkv_ref[:, 2 * D:3 * D].T

            def rows(i, carry):
                r0 = pl.multiple_of(i * r1, r1)
                x = x_ref[pl.ds(r0, r1), :].astype(f32)
                h = _ln(x) * (1.0 + mod_s[0:1, D:2 * D]) + mod_s[0:1, 0:D]
                hb = h.astype(bf16)
                q = jnp.dot(hb, wqkv_ref[:, 0:D], preferred_element_type=f32)
                q_s[pl.ds(r0, r1), :] = (q * QSCALE).astype(bf16)
                k = jnp.dot(hb, wqkv_ref[:, D:2 * D], preferred_element_type=f32)
                k_s[pl.ds(r0, r1), :] = k.astype(bf16)
                vT = lax.dot_general(wvT, hb, NT, preferred_element_type=f32)
                vT_s[:, pl.ds(r0, r1)] = vT.astype(bf16)
                return carry
            lax.fori_loop(0, S // r1, rows, 0)

        q0 = pl.multiple_of(step_id * bq, bq)
        lane = lax.broadcasted_iota(jnp.int32, (bq, 128), 1)

        def qm_of(h):
            g = h // 8
            j = h % 8
            goff = pl.multiple_of(g * 128, 128)
            qg = q_s[pl.ds(q0, bq), pl.ds(goff, 128)]
            return goff, jnp.where(lane // 16 == j, qg, jnp.zeros_like(qg))

        def qk_chunk(goff, qm, c, s_ref, m):
            s = lax.dot_general(k_s[c * kc:(c + 1) * kc, pl.ds(goff, 128)], qm, NT, preferred_element_type=f32)
            s_ref[c * kc:(c + 1) * kc, :] = s
            mc = jnp.max(s.reshape(kc // 8, 8, bq), axis=0)
            return mc if m is None else jnp.maximum(m, mc)

        def pv_chunk(hoff, c, s_ref, m, l, acc):
            p = jnp.exp2(s_ref[c * kc:(c + 1) * kc, :].reshape(kc // 8, 8, bq) - m[None])
            ls = jnp.sum(p, axis=0)
            l = ls if l is None else l + ls
            pv = jnp.dot(vT_s[pl.ds(hoff, 16), c * kc:(c + 1) * kc], p.reshape(kc, bq).astype(bf16),
                         preferred_element_type=f32)
            acc = pv if acc is None else acc + pv
            return l, acc

        def step(hn, hc, sn_ref, sc_ref, m_cur):
            if hn is not None:
                goff, qm = qm_of(hn)
            if hc is not None:
                hoff = pl.multiple_of(hc * 16, 16)
            m = None; l = None; acc = None
            for c in range(nc):
                if hn is not None:
                    m = qk_chunk(goff, qm, c, sn_ref, m)
                if hc is not None:
                    l, acc = pv_chunk(hoff, c, sc_ref, m_cur, l, acc)
            if hc is not None:
                lsum = jnp.sum(l, axis=0, keepdims=True)
                oT_s[pl.ds(hoff, 16), :] = acc / lsum
            if hn is not None:
                return jnp.broadcast_to(jnp.max(m, axis=0, keepdims=True), (8, bq))
            return None

        mA = step(0, None, sA, None, None)

        def body(i, mA):
            h = 2 * i
            mB = step(h + 1, h, sB, sA, mA)
            mA = step(h + 2, h + 1, sA, sB, mB)
            return mA
        mA = lax.fori_loop(0, H // 2 - 1, body, mA)
        mB = step(H - 1, H - 2, sB, sA, mA)
        step(None, H - 1, None, sB, mB)

        b1 = b1_ref[...].astype(f32).reshape(1, F)
        b2 = b2_ref[...].astype(f32).reshape(1, D)

        def tail(i, carry):
            r0 = pl.multiple_of(i * r2, r2)
            oT = oT_s[:, pl.ds(r0, r2)].astype(bf16)
            attn = lax.dot_general(oT, wo_ref[...], TN, preferred_element_type=f32)
            x1 = xq_ref[pl.ds(r0, r2), :].astype(f32) + mod_s[0:1, 2 * D:3 * D] * attn
            h = _ln(x1) * (1.0 + mod_s[0:1, 4 * D:5 * D]) + mod_s[0:1, 3 * D:4 * D]
            h1 = jnp.dot(h.astype(bf16), w1_ref[...], preferred_element_type=f32) + b1
            h1 = jnp.maximum(h1, 0.0)
            h1 = (h1 * h1).astype(bf16)
            y = jnp.dot(h1, w2_ref[...], preferred_element_type=f32) + b2
            o_ref[pl.ds(r0, r2), :] = (x1 + mod_s[0:1, 5 * D:6 * D] * y).astype(o_ref.dtype)
            return carry
        lax.fori_loop(0, bq // r2, tail, 0)

    full = lambda shape: pl.BlockSpec(shape, lambda i: (0,) * len(shape))
    return functools.partial(
        pl.pallas_call,
        kernel,
        grid=(nq,),
        in_specs=[full((S, D)), pl.BlockSpec((bq, D), lambda i: (i, 0)), full((D, 3 * D)), full((D, D)),
                  full((D, F)), full((F,)), full((F, D)), full((D,)), full((1, D)), full((D, 6 * D))],
        out_specs=pl.BlockSpec((bq, D), lambda i: (i, 0)),
        scratch_shapes=[pltpu.VMEM((8, 6 * D), f32), pltpu.VMEM((S, D), bf16), pltpu.VMEM((S, D), bf16),
                        pltpu.VMEM((D, S), bf16), pltpu.VMEM((S, bq), f32), pltpu.VMEM((S, bq), f32),
                        pltpu.VMEM((D, bq), f32)],
        compiler_params=pltpu.CompilerParams(vmem_limit_bytes=100 * 1024 * 1024,
                                             dimension_semantics=("arbitrary",)),
        name="fused_adaln_block",
    )


def _build(**kw):
    def fn(A_x, A_wqkv, A_wo, B_x, B_w1, B_b1, B_w2, B_b2, c, w_mod):
        x = A_x.reshape(S, D)
        out = make_kernel(**kw)(out_shape=jax.ShapeDtypeStruct((S, D), A_x.dtype))(
            x, x, A_wqkv, A_wo, B_w1, B_b1, B_w2, B_b2, c, w_mod)
        return out.reshape(A_x.shape)
    return fn


@jax.jit
def pallas_adaLN_cond__mha_block__dense_activation_squared_relu__prompt_kernel(
    A_x: jax.Array,
    A_wqkv: jax.Array,
    A_wo: jax.Array,
    B_x: jax.Array,
    B_w1: jax.Array,
    B_b1: jax.Array,
    B_w2: jax.Array,
    B_b2: jax.Array,
    c: jax.Array,
    w_mod: jax.Array,
):
    return _build()(A_x, A_wqkv, A_wo, B_x, B_w1, B_b1, B_w2, B_b2, c, w_mod)
```

```python
import functools
import numpy as np
import jax, jax.numpy as jnp
from jax import lax
from jax.experimental import pallas as pl
from jax.experimental.pallas import tpu as pltpu

S, D, H, DH, F = 2048, 512, 32, 16, 1792
QSCALE = 0.25 * 1.4426950408889634
EPS = 1e-5
NT = (((1,), (1,)), ((), ()))
TN = (((0,), (0,)), ((), ()))
f32 = jnp.float32
bf16 = jnp.bfloat16
BOUND_SHIFT = 32.0
L_MIN = float(2.0 ** -80)


def _ln(x):
    m = jnp.mean(x, axis=-1, keepdims=True)
    d = x - m
    v = jnp.mean(d * d, axis=-1, keepdims=True)
    return d * lax.rsqrt(v + EPS)


def make_kernel(bq=512, kc=128, lag=2, hu=8, r0=512, r1=512, r2=256, peel=False):
    nq = S // bq
    nc = S // kc
    n0 = S // r0
    n2 = S // r2

    def kernel(x_hbm, wqkv_hbm, wo_hbm, w1_hbm, b1_ref, w2_hbm, b2_ref, c_ref, wmod_hbm,
               o_hbm,
               x_ref, wqkv_ref, wo_ref, w1_ref, w2_ref, wmod_ref,
               mod_s, h_s, q_s, k_s, vT_s, qn_s, m_s, oT_s, x1_s, out_s, sems, osems):
        cp_mod1 = pltpu.make_async_copy(wmod_hbm.at[:, pl.ds(0, 2 * D)], wmod_ref.at[:, pl.ds(0, 2 * D)], sems.at[0])
        cp_x = [pltpu.make_async_copy(x_hbm.at[pl.ds(i * r0, r0), :], x_ref.at[pl.ds(i * r0, r0), :], sems.at[1 + i])
                for i in range(n0)]
        cp_wqkv = pltpu.make_async_copy(wqkv_hbm, wqkv_ref, sems.at[1 + n0])
        cp_mod2 = pltpu.make_async_copy(wmod_hbm.at[:, pl.ds(2 * D, 4 * D)], wmod_ref.at[:, pl.ds(2 * D, 4 * D)], sems.at[2 + n0])
        cp_wo = pltpu.make_async_copy(wo_hbm, wo_ref, sems.at[3 + n0])
        cp_w1 = pltpu.make_async_copy(w1_hbm, w1_ref, sems.at[4 + n0])
        cp_w2 = pltpu.make_async_copy(w2_hbm, w2_ref, sems.at[5 + n0])
        cp_mod1.start()
        for cp in cp_x:
            cp.start()
        cp_wqkv.start()

        c = c_ref[...].astype(f32)
        sc = jnp.broadcast_to(c * jax.nn.sigmoid(c), (16, D)).astype(bf16)
        cp_mod1.wait()
        mod1 = jnp.dot(sc, wmod_ref[:, 0:2 * D], preferred_element_type=f32)
        sa = mod1[0:1, 0:D]
        ca1 = 1.0 + mod1[0:1, D:2 * D]
        for i in range(n0):
            cp_x[i].wait()
            x = x_ref[i * r0:(i + 1) * r0, :].astype(f32)
            h_s[i * r0:(i + 1) * r0, :] = (_ln(x) * ca1 + sa).astype(bf16)
        cp_wqkv.wait()
        cp_mod2.start()
        cp_wo.start()
        cp_w1.start()
        cp_w2.start()

        wvT = wqkv_ref[:, 2 * D:3 * D].T
        ehead = (lax.broadcasted_iota(jnp.int32, (H, D), 1) // DH
                 == lax.broadcasted_iota(jnp.int32, (H, D), 0)).astype(bf16)

        def rows(i, kmax):
            rr = pl.multiple_of(i * r1, r1)
            hb = h_s[pl.ds(rr, r1), :]
            q = jnp.dot(hb, wqkv_ref[:, 0:D], preferred_element_type=f32) * QSCALE
            q_s[pl.ds(rr, r1), :] = q.astype(bf16)
            k = jnp.dot(hb, wqkv_ref[:, D:2 * D], preferred_element_type=f32)
            k_s[pl.ds(rr, r1), :] = k.astype(bf16)
            vT = lax.dot_general(wvT, hb, NT, preferred_element_type=f32)
            vT_s[:, pl.ds(rr, r1)] = vT.astype(bf16)
            qn_s[:, pl.ds(rr, r1)] = lax.dot_general(ehead, (q * q).astype(bf16), NT, preferred_element_type=f32)
            kn = lax.dot_general(ehead, (k * k).astype(bf16), NT, preferred_element_type=f32)
            return jnp.maximum(kmax, kn)
        kmax = lax.fori_loop(0, S // r1, rows, jnp.zeros((H, r1), f32))
        kmax = jnp.max(kmax, axis=1, keepdims=True)
        m_s[...] = jnp.sqrt(qn_s[...] * kmax) * 1.01 - BOUND_SHIFT

        lane = lax.broadcasted_iota(jnp.int32, (bq, 128), 1)
        nit = nq * (H // hu)

        def heads(it, lmin):
            qb = it // (H // hu)
            hg = it % (H // hu)
            q0 = pl.multiple_of(qb * bq, bq)
            items = []
            st = {}
            for u in range(hu):
                h = hg * hu + u
                goff = pl.multiple_of((hg * hu + u) // 8 * 128, 128)
                hoff = pl.multiple_of(h * DH, DH)
                qg = q_s[pl.ds(q0, bq), pl.ds(goff, 128)]
                if hu >= 8:
                    qm = jnp.where(lane // DH == (u % 8), qg, jnp.zeros_like(qg))
                else:
                    qm = jnp.where(lane // DH == h % 8, qg, jnp.zeros_like(qg))
                m = jnp.broadcast_to(m_s[pl.ds(h, 1), pl.ds(q0, bq)], (8, bq))
                st[u] = dict(goff=goff, hoff=hoff, qm=qm, m=m, l=None, acc=None)
                for cc in range(nc):
                    items.append((u, cc))
            svals = {}
            n = len(items)
            for t in range(n + lag):
                if t < n:
                    u, cc = items[t]
                    d = st[u]
                    svals[t] = lax.dot_general(k_s[cc * kc:(cc + 1) * kc, pl.ds(d['goff'], 128)], d['qm'], NT,
                                               preferred_element_type=f32)
                if t - lag >= 0:
                    u, cc = items[t - lag]
                    d = st[u]
                    p = jnp.exp2(svals.pop(t - lag).reshape(kc // 8, 8, bq) - d['m'][None])
                    ls = jnp.sum(p, axis=0)
                    d['l'] = ls if d['l'] is None else d['l'] + ls
                    r = jnp.dot(vT_s[pl.ds(d['hoff'], DH), cc * kc:(cc + 1) * kc], p.reshape(kc, bq).astype(bf16),
                                preferred_element_type=f32)
                    d['acc'] = r if d['acc'] is None else d['acc'] + r
                    if cc == nc - 1:
                        lsum = jnp.sum(d['l'], axis=0, keepdims=True)
                        lmin = jnp.minimum(lmin, lsum)
                        oT_s[pl.ds(d['hoff'], DH), pl.ds(q0, bq)] = (d['acc'] * (1.0 / lsum)).astype(bf16)
            return lmin
        lmin = lax.fori_loop(0, nit, heads, jnp.full((1, bq), 1.0, f32))
        unsafe = jnp.logical_not(jnp.min(lmin) >= L_MIN)

        @pl.when(unsafe)
        def _():
            lane_f = lax.broadcasted_iota(jnp.int32, (128, 128), 1)

            def one(it, carry):
                qb = it // H
                h = it % H
                q0 = pl.multiple_of(qb * 128, 128)
                goff = pl.multiple_of(h // 8 * 128, 128)
                hoff = pl.multiple_of(h * DH, DH)
                qg = q_s[pl.ds(q0, 128), pl.ds(goff, 128)]
                qm = jnp.where(lane_f // DH == h % 8, qg, jnp.zeros_like(qg))
                s = lax.dot_general(k_s[:, pl.ds(goff, 128)], qm, NT, preferred_element_type=f32)
                p = jnp.exp2(s - jnp.max(s, axis=0, keepdims=True))
                l = jnp.sum(p, axis=0, keepdims=True)
                o = jnp.dot(vT_s[pl.ds(hoff, DH), :], p.astype(bf16), preferred_element_type=f32)
                oT_s[pl.ds(hoff, DH), pl.ds(q0, 128)] = (o / l).astype(bf16)
                return carry
            lax.fori_loop(0, (S // 128) * H, one, 0)

        cp_mod2.wait()
        cp_wo.wait()
        cp_w1.wait()
        cp_w2.wait()
        mod2 = jnp.dot(sc, wmod_ref[:, 2 * D:6 * D], preferred_element_type=f32)
        mod_s[...] = mod2[0:8]
        b1 = b1_ref[...].astype(f32).reshape(1, F)
        b2 = b2_ref[...].astype(f32).reshape(1, D)

        def proj_ln(rr):
            attn = lax.dot_general(oT_s[:, pl.ds(rr, r2)], wo_ref[...], TN, preferred_element_type=f32)
            x1 = x_ref[pl.ds(rr, r2), :].astype(f32) + mod_s[0:1, 0:D] * attn
            x1_s[pl.ds(rr, r2), :] = x1
            h = _ln(x1) * (1.0 + mod_s[0:1, 2 * D:3 * D]) + mod_s[0:1, D:2 * D]
            h_s[pl.ds(rr, r2), :] = h.astype(bf16)

        def ffn(rr):
            h1 = jnp.dot(h_s[pl.ds(rr, r2), :], w1_ref[...], preferred_element_type=f32) + b1
            h1 = jnp.maximum(h1, 0.0)
            h1 = (h1 * h1).astype(bf16)
            y = jnp.dot(h1, w2_ref[...], preferred_element_type=f32) + b2
            out_s[pl.ds(rr, r2), :] = (x1_s[pl.ds(rr, r2), :] + mod_s[0:1, 3 * D:4 * D] * y).astype(out_s.dtype)

        def out_copy(i):
            rr = pl.multiple_of(i * r2, r2)
            return pltpu.make_async_copy(out_s.at[pl.ds(rr, r2), :], o_hbm.at[pl.ds(rr, r2), :], osems.at[i])

        proj_ln(0)

        def tail(i, carry):
            rr = pl.multiple_of(i * r2, r2)
            rn = pl.multiple_of(jnp.minimum(i + 1, n2 - 1) * r2, r2)
            ffn(rr)
            proj_ln(rn)
            out_copy(i).start()
            return carry
        if peel:
            lax.fori_loop(0, n2 - 1, tail, 0)
            ffn((n2 - 1) * r2)
            out_copy(n2 - 1).start()
        else:
            lax.fori_loop(0, n2, tail, 0)
        for i in range(n2):
            out_copy(i).wait()

    any_spec = pl.BlockSpec(memory_space=pl.ANY)
    vm = pl.BlockSpec(memory_space=pltpu.VMEM)
    return functools.partial(
        pl.pallas_call,
        kernel,
        in_specs=[any_spec, any_spec, any_spec, any_spec, vm, any_spec, vm, vm, any_spec],
        out_specs=any_spec,
        scratch_shapes=[
            pltpu.VMEM((S, D), bf16), pltpu.VMEM((D, 3 * D), bf16), pltpu.VMEM((D, D), bf16),
            pltpu.VMEM((D, F), bf16), pltpu.VMEM((F, D), bf16), pltpu.VMEM((D, 6 * D), bf16),
            pltpu.VMEM((8, 4 * D), f32), pltpu.VMEM((S, D), bf16), pltpu.VMEM((S, D), bf16),
            pltpu.VMEM((S, D), bf16), pltpu.VMEM((D, S), bf16), pltpu.VMEM((H, S), f32), pltpu.VMEM((H, S), f32),
            pltpu.VMEM((D, S), bf16), pltpu.VMEM((S, D), f32), pltpu.VMEM((S, D), bf16),
            pltpu.SemaphoreType.DMA((6 + n0,)), pltpu.SemaphoreType.DMA((n2,)),
        ],
        compiler_params=pltpu.CompilerParams(vmem_limit_bytes=100 * 1024 * 1024),
        name="fused_adaln_block",
    )


def _build(**kw):
    def fn(A_x, A_wqkv, A_wo, B_x, B_w1, B_b1, B_w2, B_b2, c, w_mod):
        x = A_x.reshape(S, D)
        out = make_kernel(**kw)(out_shape=jax.ShapeDtypeStruct((S, D), A_x.dtype))(
            x, A_wqkv, A_wo, B_w1, B_b1, B_w2, B_b2, c, w_mod)
        return out.reshape(A_x.shape)
    return fn


@jax.jit
def pallas_adaLN_cond__mha_block__dense_activation_squared_relu__prompt_kernel(
    A_x: jax.Array,
    A_wqkv: jax.Array,
    A_wo: jax.Array,
    B_x: jax.Array,
    B_w1: jax.Array,
    B_b1: jax.Array,
    B_w2: jax.Array,
    B_b2: jax.Array,
    c: jax.Array,
    w_mod: jax.Array,
):
    return _build(hu=16, peel=True)(A_x, A_wqkv, A_wo, B_x, B_w1, B_b1, B_w2, B_b2, c, w_mod)
```

```python
import functools
import numpy as np
import jax, jax.numpy as jnp
from jax import lax
from jax.experimental import pallas as pl
from jax.experimental.pallas import tpu as pltpu

S, D, H, DH, F = 2048, 512, 32, 16, 1792
QSCALE = 0.25 * 1.4426950408889634
EPS = 1e-5
NT = (((1,), (1,)), ((), ()))
TN = (((0,), (0,)), ((), ()))
f32 = jnp.float32
bf16 = jnp.bfloat16
BOUND_SHIFT = 32.0
L_MIN = float(2.0 ** -80)


def _ln(x):
    m = jnp.mean(x, axis=-1, keepdims=True)
    d = x - m
    v = jnp.mean(d * d, axis=-1, keepdims=True)
    return d * lax.rsqrt(v + EPS)


def make_kernel(bq=512, kc=128, lag=2, hu=8, r1=512, r2=256, peel=False, dmo=0):
    nq = S // bq
    nc = S // kc
    n1 = S // r1
    n2 = S // r2

    def kernel(x_hbm, wqkv_hbm, wo_hbm, w1_hbm, b1_ref, w2_hbm, b2_ref, c_ref, wmod_hbm,
               o_hbm,
               x_ref, wqkv_ref, wo_ref, w1_ref, w2_ref, wmod_ref,
               mod_s, wT_s, qT_s, k_s, vT_s, qn_s, kn_s, oT_s, out_s, h_s, sp_s, x1a_s, x1b_s, h2a_s, h2b_s,
               sems, xsems, osems):
        x1_s = (x1a_s, x1b_s)
        h2_s = (h2a_s, h2b_s)
        def cols(hbm, vmem, start, size, sem):
            return pltpu.make_async_copy(hbm.at[:, pl.ds(start, size)], vmem.at[:, pl.ds(start, size)], sem)

        def x_copy(i):
            rr = pl.multiple_of(i * r1, r1)
            return pltpu.make_async_copy(x_hbm.at[pl.ds(rr, r1), :], x_ref.at[pl.ds(rr, r1), :], xsems.at[i])

        cp_mod1 = cols(wmod_hbm, wmod_ref, 0, 2 * D, sems.at[0])
        cp_wk = cols(wqkv_hbm, wqkv_ref, D, D, sems.at[1])
        cp_wq = cols(wqkv_hbm, wqkv_ref, 0, D, sems.at[2])
        cp_wv = cols(wqkv_hbm, wqkv_ref, 2 * D, D, sems.at[3])
        cp_mod2 = cols(wmod_hbm, wmod_ref, 2 * D, 4 * D, sems.at[4])
        cp_wo = pltpu.make_async_copy(wo_hbm, wo_ref, sems.at[5])
        cp_w1 = pltpu.make_async_copy(w1_hbm, w1_ref, sems.at[6])
        cp_w2 = pltpu.make_async_copy(w2_hbm, w2_ref, sems.at[7])
        cp_mod1.start()
        x_copy(0).start()
        cp_wk.start()
        cp_wq.start()
        if dmo == 0:
            cp_wv.start()
            for i in range(1, n1):
                x_copy(i).start()

        c = c_ref[...].astype(f32)
        sc = jnp.broadcast_to(c * jax.nn.sigmoid(c), (16, D)).astype(bf16)
        cp_mod1.wait()
        mod1 = jnp.dot(sc, wmod_ref[:, 0:2 * D], preferred_element_type=f32)
        sa = mod1[0:1, 0:D]
        ca1 = 1.0 + mod1[0:1, D:2 * D]

        def ln1(i):
            x = x_ref[i * r1:(i + 1) * r1, :].astype(f32)
            h_s[i * r1:(i + 1) * r1, :] = (_ln(x) * ca1 + sa).astype(bf16)

        ehead = (lax.broadcasted_iota(jnp.int32, (H, D), 1) // DH
                 == lax.broadcasted_iota(jnp.int32, (H, D), 0)).astype(bf16)

        def k_part(rr, kmax):
            k = jnp.dot(h_s[pl.ds(rr, r1), :], wqkv_ref[:, D:2 * D], preferred_element_type=f32)
            k_s[pl.ds(rr, r1), :] = k.astype(bf16)
            kn = lax.dot_general(ehead, (k * k).astype(bf16), NT, preferred_element_type=f32)
            return jnp.maximum(kmax, kn)

        def q_part(rr):
            qT = lax.dot_general(wT_s[0:D, :], h_s[pl.ds(rr, r1), :], NT, preferred_element_type=f32) * QSCALE
            qT_s[:, pl.ds(rr, r1)] = qT.astype(bf16)
            qn2 = jnp.dot(ehead, (qT * qT).astype(bf16), preferred_element_type=f32)
            qn_s[:, pl.ds(rr, r1)] = jnp.sqrt(qn2)

        def v_part(rr):
            vT = lax.dot_general(wT_s[D:2 * D, :], h_s[pl.ds(rr, r1), :], NT, preferred_element_type=f32)
            vT_s[:, pl.ds(rr, r1)] = vT.astype(bf16)

        x_copy(0).wait()
        if dmo == 1:
            cp_wv.start()
            for i in range(1, n1):
                x_copy(i).start()
        ln1(0)
        cp_wk.wait()
        if dmo == 2:
            cp_wv.start()
            x_copy(1).start()
        cp_wq.wait()
        if dmo >= 3:
            cp_wv.start()
            x_copy(1).start()
        wT_s[0:D, :] = wqkv_ref[:, 0:D].T
        kmax = k_part(0, jnp.zeros((H, r1), f32))
        cp_wv.wait()
        x_copy(1).wait()
        if dmo >= 2:
            for i in range(2, n1):
                x_copy(i).start()
        wT_s[D:2 * D, :] = wqkv_ref[:, 2 * D:3 * D].T
        ln1(1)
        q_part(0)
        for i in range(2, n1):
            x_copy(i).wait()
        cp_mod2.start()
        cp_wo.start()
        cp_w1.start()
        cp_w2.start()
        for i in range(2, n1):
            ln1(i)
        v_part(0)

        def rows(i, kmax):
            rr = pl.multiple_of(i * r1, r1)
            kmax = k_part(rr, kmax)
            q_part(rr)
            v_part(rr)
            return kmax
        kmax = lax.fori_loop(1, n1, rows, kmax)
        kn_s[...] = jnp.broadcast_to(jnp.sqrt(jnp.max(kmax, axis=1, keepdims=True)) * 1.01, (H, 128))

        G = H // hu
        nit = nq * G

        def pv_stage(s, d, cc):
            p = jnp.exp2(s.reshape(kc // 8, 8, bq) - d['m'][None])
            ls = jnp.sum(p, axis=0)
            d['l'] = ls if d['l'] is None else d['l'] + ls
            r = jnp.dot(vT_s[pl.ds(d['hoff'], DH), cc * kc:(cc + 1) * kc], p.reshape(kc, bq).astype(bf16),
                        preferred_element_type=f32)
            d['acc'] = r if d['acc'] is None else d['acc'] + r

        def finalize(d, lmin):
            lsum = jnp.sum(d['l'], axis=0, keepdims=True)
            oT_s[pl.ds(d['hoff'], DH), pl.ds(d['q0'], bq)] = (d['acc'] * (1.0 / lsum)).astype(bf16)
            return jnp.minimum(lmin, lsum)

        def prev_state(itp, l, acc, m):
            hp = (itp % G) * hu + (hu - 1)
            return dict(hoff=pl.multiple_of(hp * DH, DH), q0=pl.multiple_of((itp // G) * bq, bq), l=l, acc=acc, m=m)

        def heads(it, carry):
            lmin, l_p, acc_p, m_p = carry
            prev = prev_state((it + nit - 1) % nit, l_p, acc_p, m_p)
            hg = it % G
            q0 = pl.multiple_of((it // G) * bq, bq)
            items = []
            st = {}
            for u in range(hu):
                h = hg * hu + u
                goff = pl.multiple_of((hg * hu + u) // 8 * 128, 128)
                hoff = pl.multiple_of(h * DH, DH)
                jj = u % 8
                parts = [qT_s[pl.ds(hoff, DH), pl.ds(q0, bq)]]
                if jj > 0:
                    parts.insert(0, jnp.zeros((DH * jj, bq), bf16))
                if jj < 7:
                    parts.append(jnp.zeros((DH * (7 - jj), bq), bf16))
                qm = jnp.concatenate(parts, axis=0)
                kn = kn_s[pl.ds(h, 1), :]
                kn = jnp.concatenate([kn] * (bq // 128), axis=1)
                m = jnp.broadcast_to(qn_s[pl.ds(h, 1), pl.ds(q0, bq)] * kn - BOUND_SHIFT, (8, bq))
                st[u] = dict(goff=goff, hoff=hoff, q0=q0, qm=qm, m=m, l=None, acc=None)
                for cc in range(nc):
                    items.append((u, cc))
            svals = {}
            n = len(items)
            for t in range(n):
                u, cc = items[t]
                d = st[u]
                svals[t] = jnp.dot(k_s[cc * kc:(cc + 1) * kc, pl.ds(d['goff'], 128)], d['qm'],
                                   preferred_element_type=f32)
                if t < lag:
                    pv_stage(sp_s[t], prev, nc - lag + t)
                    if t == lag - 1:
                        lmin = finalize(prev, lmin)
                else:
                    u, cc = items[t - lag]
                    pv_stage(svals.pop(t - lag), st[u], cc)
                    if cc == nc - 1:
                        lmin = finalize(st[u], lmin)
            for t in range(lag):
                sp_s[t] = svals.pop(n - lag + t)
            d = st[hu - 1]
            return lmin, d['l'], d['acc'], d['m']

        sp_s[...] = jnp.zeros(sp_s.shape, f32)
        init = (jnp.full((1, bq), 1.0, f32), jnp.zeros((8, bq), f32), jnp.zeros((DH, bq), f32),
                jnp.zeros((8, bq), f32))
        lmin, l_p, acc_p, m_p = lax.fori_loop(0, nit, heads, init)
        last = prev_state(nit - 1, l_p, acc_p, m_p)
        for t in range(lag):
            pv_stage(sp_s[t], last, nc - lag + t)
        lmin = finalize(last, lmin)
        unsafe = jnp.logical_not(jnp.min(lmin) >= L_MIN)

        @pl.when(unsafe)
        def _():
            row_f = lax.broadcasted_iota(jnp.int32, (128, 128), 0)

            def one(it, carry):
                qb = it // H
                h = it % H
                q0 = pl.multiple_of(qb * 128, 128)
                goff = pl.multiple_of(h // 8 * 128, 128)
                hoff = pl.multiple_of(h * DH, DH)
                qg = qT_s[pl.ds(goff, 128), pl.ds(q0, 128)]
                qm = jnp.where(row_f // DH == h % 8, qg, jnp.zeros_like(qg))
                s = jnp.dot(k_s[:, pl.ds(goff, 128)], qm, preferred_element_type=f32)
                p = jnp.exp2(s - jnp.max(s, axis=0, keepdims=True))
                l = jnp.sum(p, axis=0, keepdims=True)
                o = jnp.dot(vT_s[pl.ds(hoff, DH), :], p.astype(bf16), preferred_element_type=f32)
                oT_s[pl.ds(hoff, DH), pl.ds(q0, 128)] = (o / l).astype(bf16)
                return carry
            lax.fori_loop(0, (S // 128) * H, one, 0)

        cp_mod2.wait()
        cp_wo.wait()
        cp_w1.wait()
        cp_w2.wait()
        mod2 = jnp.dot(sc, wmod_ref[:, 2 * D:6 * D], preferred_element_type=f32)
        mod_s[...] = mod2[0:8]
        b1 = b1_ref[...].astype(f32).reshape(1, F)
        b2 = b2_ref[...].astype(f32).reshape(1, D)

        def proj_ln(i, slot):
            rr = pl.multiple_of(i * r2, r2)
            attn = lax.dot_general(oT_s[:, pl.ds(rr, r2)], wo_ref[...], TN, preferred_element_type=f32)
            x1 = x_ref[pl.ds(rr, r2), :].astype(f32) + mod_s[0:1, 0:D] * attn
            x1_s[slot][...] = x1
            h = _ln(x1) * (1.0 + mod_s[0:1, 2 * D:3 * D]) + mod_s[0:1, D:2 * D]
            h2_s[slot][...] = h.astype(bf16)

        def out_copy(i):
            rr = pl.multiple_of(i * r2, r2)
            return pltpu.make_async_copy(out_s.at[pl.ds(rr, r2), :], o_hbm.at[pl.ds(rr, r2), :], osems.at[i])

        def ffn(i, slot):
            rr = pl.multiple_of(i * r2, r2)
            h1 = jnp.dot(h2_s[slot][...], w1_ref[...], preferred_element_type=f32) + b1
            h1 = jnp.maximum(h1, 0.0)
            h1 = (h1 * h1).astype(bf16)
            y = jnp.dot(h1, w2_ref[...], preferred_element_type=f32) + b2
            out_s[pl.ds(rr, r2), :] = (x1_s[slot][...] + mod_s[0:1, 3 * D:4 * D] * y).astype(out_s.dtype)

        def tail(j, carry):
            i = 2 * j
            proj_ln(i + 1, 1)
            ffn(i, 0)
            out_copy(i).start()
            proj_ln(jnp.minimum(i + 2, n2 - 1), 0)
            ffn(i + 1, 1)
            out_copy(i + 1).start()
            return carry
        proj_ln(0, 0)
        if peel:
            lax.fori_loop(0, n2 // 2 - 1, tail, 0)
            proj_ln(n2 - 1, 1)
            ffn(n2 - 2, 0)
            out_copy(n2 - 2).start()
            ffn(n2 - 1, 1)
            out_copy(n2 - 1).start()
        else:
            lax.fori_loop(0, n2 // 2, tail, 0)
        for i in range(n2):
            out_copy(i).wait()

    any_spec = pl.BlockSpec(memory_space=pl.ANY)
    vm = pl.BlockSpec(memory_space=pltpu.VMEM)
    return functools.partial(
        pl.pallas_call,
        kernel,
        in_specs=[any_spec, any_spec, any_spec, any_spec, vm, any_spec, vm, vm, any_spec],
        out_specs=any_spec,
        scratch_shapes=[
            pltpu.VMEM((S, D), bf16), pltpu.VMEM((D, 3 * D), bf16), pltpu.VMEM((D, D), bf16),
            pltpu.VMEM((D, F), bf16), pltpu.VMEM((F, D), bf16), pltpu.VMEM((D, 6 * D), bf16),
            pltpu.VMEM((8, 4 * D), f32), pltpu.VMEM((2 * D, D), bf16), pltpu.VMEM((D, S), bf16),
            pltpu.VMEM((S, D), bf16), pltpu.VMEM((D, S), bf16), pltpu.VMEM((H, S), f32),
            pltpu.VMEM((H, 128), f32), pltpu.VMEM((D, S), bf16), pltpu.VMEM((S, D), bf16),
            pltpu.VMEM((S, D), bf16), pltpu.VMEM((lag, kc, bq), f32), pltpu.VMEM((r2, D), f32),
            pltpu.VMEM((r2, D), f32), pltpu.VMEM((r2, D), bf16), pltpu.VMEM((r2, D), bf16),
            pltpu.SemaphoreType.DMA((8,)), pltpu.SemaphoreType.DMA((n1,)), pltpu.SemaphoreType.DMA((n2,)),
        ],
        compiler_params=pltpu.CompilerParams(vmem_limit_bytes=100 * 1024 * 1024),
        name="fused_adaln_block",
    )


def _build(**kw):
    def fn(A_x, A_wqkv, A_wo, B_x, B_w1, B_b1, B_w2, B_b2, c, w_mod):
        x = A_x.reshape(S, D)
        out = make_kernel(**kw)(out_shape=jax.ShapeDtypeStruct((S, D), A_x.dtype))(
            x, A_wqkv, A_wo, B_w1, B_b1, B_w2, B_b2, c, w_mod)
        return out.reshape(A_x.shape)
    return fn


@jax.jit
def pallas_adaLN_cond__mha_block__dense_activation_squared_relu__prompt_kernel(
    A_x: jax.Array,
    A_wqkv: jax.Array,
    A_wo: jax.Array,
    B_x: jax.Array,
    B_w1: jax.Array,
    B_b1: jax.Array,
    B_w2: jax.Array,
    B_b2: jax.Array,
    c: jax.Array,
    w_mod: jax.Array,
):
    return _build(hu=16, r2=128, dmo=3)(A_x, A_wqkv, A_wo, B_x, B_w1, B_b1, B_w2, B_b2, c, w_mod)
```

```python
import functools
import jax
import jax.numpy as jnp
from jax import lax
from jax.experimental import pallas as pl
from jax.experimental.pallas import tpu as pltpu

S, D, H, DH, F = 2048, 512, 32, 16, 1792
QSCALE = 0.25 * 1.4426950408889634
EPS = 1e-5
BOUND_SLACK = 1.01
L_MIN = float(2.0 ** -90)
NT = (((1,), (1,)), ((), ()))
TN = (((0,), (0,)), ((), ()))
f32 = jnp.float32
bf16 = jnp.bfloat16


def _ln(x):
    m = jnp.mean(x, axis=-1, keepdims=True)
    d = x - m
    v = jnp.mean(d * d, axis=-1, keepdims=True)
    return d * lax.rsqrt(v + EPS)


def make_kernel(bq=512, kc=128, lag=2, hu=16, r1=512, r2=128, lp=64):
    nq = S // bq
    nc = S // kc
    n1 = S // r1
    n2 = S // r2
    G = H // hu
    nit = nq * G

    def kernel(x_hbm, wqkv_hbm, wo_hbm, w1_hbm, b1_hbm, w2_hbm, b2_hbm, c_hbm, wmod_hbm,
               o_hbm,
               x_ref, wqkv_ref, wo_ref, w1_ref, w2_ref, wmod_ref,
               mod_s, wT_s, qT_s, k_s, vT_s, qn_s, kn_s, oT_s, out_s, h_s, sp_s, x1a_s, x1b_s, h2a_s, h2b_s,
               c_ref, b1_ref, b2_ref, sems, xsems, osems):
        x1_s = (x1a_s, x1b_s)
        h2_s = (h2a_s, h2b_s)

        def cols(hbm, vmem, start, size, sem):
            return pltpu.make_async_copy(hbm.at[:, pl.ds(start, size)], vmem.at[:, pl.ds(start, size)], sem)

        def x_copy(i):
            return pltpu.make_async_copy(x_hbm.at[pl.ds(i * r1, r1), :], x_ref.at[pl.ds(i * r1, r1), :], xsems.at[i])

        cp_mod1 = cols(wmod_hbm, wmod_ref, 0, 2 * D, sems.at[0])
        cp_wk = cols(wqkv_hbm, wqkv_ref, D, D, sems.at[1])
        cp_wq = cols(wqkv_hbm, wqkv_ref, 0, D, sems.at[2])
        cp_wv = cols(wqkv_hbm, wqkv_ref, 2 * D, D, sems.at[3])
        cp_mod2 = cols(wmod_hbm, wmod_ref, 2 * D, 4 * D, sems.at[4])
        cp_wo = pltpu.make_async_copy(wo_hbm, wo_ref, sems.at[5])
        cp_w1 = pltpu.make_async_copy(w1_hbm, w1_ref, sems.at[6])
        cp_w2 = pltpu.make_async_copy(w2_hbm, w2_ref, sems.at[7])
        cp_c = pltpu.make_async_copy(c_hbm, c_ref, sems.at[8])
        cp_b1 = pltpu.make_async_copy(b1_hbm, b1_ref, sems.at[9])
        cp_b2 = pltpu.make_async_copy(b2_hbm, b2_ref, sems.at[10])
        cp_c.start()
        cp_mod1.start()
        x_copy(0).start()
        cp_wk.start()
        cp_wq.start()

        cp_c.wait()
        c = c_ref[...].astype(f32)
        sc = jnp.broadcast_to(c * jax.nn.sigmoid(c), (16, D)).astype(bf16)
        cp_mod1.wait()
        mod1 = jnp.dot(sc, wmod_ref[:, 0:2 * D], preferred_element_type=f32)
        sa = mod1[0:1, 0:D]
        ca1 = 1.0 + mod1[0:1, D:2 * D]

        def ln_rows(r, n):
            x = x_ref[r:r + n, :].astype(f32)
            h_s[r:r + n, :] = (_ln(x) * ca1 + sa).astype(bf16)

        ehead = (lax.broadcasted_iota(jnp.int32, (H, D), 1) // DH
                 == lax.broadcasted_iota(jnp.int32, (H, D), 0)).astype(bf16)

        def k_rows(r, n):
            k = jnp.dot(h_s[pl.ds(r, n), :], wqkv_ref[:, D:2 * D], preferred_element_type=f32)
            k_s[pl.ds(r, n), :] = k.astype(bf16)
            return k

        def k_norm(k):
            return lax.dot_general(ehead, (k * k).astype(bf16), NT, preferred_element_type=f32)

        def q_cols(r, n):
            qT = lax.dot_general(wT_s[0:D, :], h_s[pl.ds(r, n), :], NT, preferred_element_type=f32) * QSCALE
            qT_s[:, pl.ds(r, n)] = qT.astype(bf16)
            qn_s[:, pl.ds(r, n)] = jnp.sqrt(jnp.dot(ehead, (qT * qT).astype(bf16), preferred_element_type=f32))

        def v_cols(r, n):
            vT = lax.dot_general(wT_s[D:2 * D, :], h_s[pl.ds(r, n), :], NT, preferred_element_type=f32)
            vT_s[:, pl.ds(r, n)] = vT.astype(bf16)

        x_copy(0).wait()
        ln_rows(0, r1)
        cp_wk.wait()
        x_copy(1).start()
        cp_wv.start()
        for i in range(2, n1):
            x_copy(i).start()
        ka = k_rows(0, r1 // 2)
        cp_wq.wait()
        wT_s[0:D, :] = wqkv_ref[:, 0:D].T
        kb = k_rows(r1 // 2, r1 // 2)
        kmax = k_norm(jnp.concatenate([ka, kb], axis=0))
        qr = r1 // 4
        cp_wv.wait()
        x_copy(1).wait()
        for t in range(4):
            q_cols(t * qr, qr)
            if t == 0:
                wT_s[D:2 * D, :] = wqkv_ref[:, 2 * D:3 * D].T
            for z in range(qr // lp):
                ln_rows(r1 + t * qr + z * lp, lp)
        for i in range(2, n1):
            x_copy(i).wait()
        cp_mod2.start()
        cp_wo.start()
        cp_b1.start()
        cp_b2.start()
        cp_w1.start()
        cp_w2.start()
        for t in range(4):
            v_cols(t * qr, qr)
            for z in range(2 * qr // lp):
                ln_rows(2 * r1 + t * 2 * qr + z * lp, lp)

        def rows(i, kmax):
            rr = pl.multiple_of(i * r1, r1)
            kmax = jnp.maximum(kmax, k_norm(k_rows(rr, r1)))
            q_cols(rr, r1)
            v_cols(rr, r1)
            return kmax
        kmax = lax.fori_loop(1, n1, rows, kmax)
        kn_s[...] = jnp.broadcast_to(jnp.sqrt(jnp.max(kmax, axis=1, keepdims=True)) * BOUND_SLACK, (H, 128))

        def pv_stage(s, d, cc):
            p = jnp.exp2(s.reshape(kc // 8, 8, bq) - d['m'][None])
            ls = jnp.sum(p, axis=0)
            d['l'] = ls if d['l'] is None else d['l'] + ls
            r = jnp.dot(vT_s[pl.ds(d['hoff'], DH), cc * kc:(cc + 1) * kc], p.reshape(kc, bq).astype(bf16),
                        preferred_element_type=f32)
            d['acc'] = r if d['acc'] is None else d['acc'] + r

        def finalize(d, lmin):
            lsum = jnp.sum(d['l'], axis=0, keepdims=True)
            oT_s[pl.ds(d['hoff'], DH), pl.ds(d['q0'], bq)] = (d['acc'] * (1.0 / lsum)).astype(bf16)
            return jnp.minimum(lmin, lsum)

        def prev_state(itp, l, acc, m):
            hp = (itp % G) * hu + (hu - 1)
            return dict(hoff=pl.multiple_of(hp * DH, DH), q0=pl.multiple_of((itp // G) * bq, bq), l=l, acc=acc, m=m)

        def heads(it, carry):
            lmin, l_p, acc_p, m_p = carry
            prev = prev_state((it + nit - 1) % nit, l_p, acc_p, m_p)
            hg = it % G
            q0 = pl.multiple_of((it // G) * bq, bq)
            items = []
            st = {}
            for u in range(hu):
                h = hg * hu + u
                goff = pl.multiple_of((hg * hu + u) // 8 * 128, 128)
                hoff = pl.multiple_of(h * DH, DH)
                jj = u % 8
                parts = [qT_s[pl.ds(hoff, DH), pl.ds(q0, bq)]]
                if jj > 0:
                    parts.insert(0, jnp.zeros((DH * jj, bq), bf16))
                if jj < 7:
                    parts.append(jnp.zeros((DH * (7 - jj), bq), bf16))
                qm = jnp.concatenate(parts, axis=0)
                kn = jnp.concatenate([kn_s[pl.ds(h, 1), :]] * (bq // 128), axis=1)
                m = jnp.broadcast_to(qn_s[pl.ds(h, 1), pl.ds(q0, bq)] * kn, (8, bq))
                st[u] = dict(goff=goff, hoff=hoff, q0=q0, qm=qm, m=m, l=None, acc=None)
                for cc in range(nc):
                    items.append((u, cc))
            svals = {}
            n = len(items)
            for t in range(n):
                u, cc = items[t]
                d = st[u]
                svals[t] = jnp.dot(k_s[cc * kc:(cc + 1) * kc, pl.ds(d['goff'], 128)], d['qm'],
                                   preferred_element_type=f32)
                if t < lag:
                    pv_stage(sp_s[t], prev, nc - lag + t)
                    if t == lag - 1:
                        lmin = finalize(prev, lmin)
                else:
                    u, cc = items[t - lag]
                    pv_stage(svals.pop(t - lag), st[u], cc)
                    if cc == nc - 1:
                        lmin = finalize(st[u], lmin)
            for t in range(lag):
                sp_s[t] = svals.pop(n - lag + t)
            d = st[hu - 1]
            return lmin, d['l'], d['acc'], d['m']

        sp_s[...] = jnp.zeros(sp_s.shape, f32)
        init = (jnp.full((1, bq), 1.0, f32), jnp.zeros((8, bq), f32), jnp.zeros((DH, bq), f32),
                jnp.zeros((8, bq), f32))
        lmin, l_p, acc_p, m_p = lax.fori_loop(0, nit, heads, init)
        last = prev_state(nit - 1, l_p, acc_p, m_p)
        for t in range(lag):
            pv_stage(sp_s[t], last, nc - lag + t)
        lmin = finalize(last, lmin)
        unsafe = jnp.logical_not(jnp.min(lmin) >= L_MIN)

        @pl.when(unsafe)
        def _():
            row_f = lax.broadcasted_iota(jnp.int32, (128, 128), 0)

            def one(it, carry):
                h = it % H
                q0 = pl.multiple_of((it // H) * 128, 128)
                goff = pl.multiple_of(h // 8 * 128, 128)
                hoff = pl.multiple_of(h * DH, DH)
                qg = qT_s[pl.ds(goff, 128), pl.ds(q0, 128)]
                qm = jnp.where(row_f // DH == h % 8, qg, jnp.zeros_like(qg))
                s = jnp.dot(k_s[:, pl.ds(goff, 128)], qm, preferred_element_type=f32)
                p = jnp.exp2(s - jnp.max(s, axis=0, keepdims=True))
                l = jnp.sum(p, axis=0, keepdims=True)
                o = jnp.dot(vT_s[pl.ds(hoff, DH), :], p.astype(bf16), preferred_element_type=f32)
                oT_s[pl.ds(hoff, DH), pl.ds(q0, 128)] = (o / l).astype(bf16)
                return carry
            lax.fori_loop(0, (S // 128) * H, one, 0)

        cp_mod2.wait()
        cp_wo.wait()
        cp_b1.wait()
        cp_b2.wait()
        cp_w1.wait()
        cp_w2.wait()
        mod_s[...] = jnp.dot(sc, wmod_ref[:, 2 * D:6 * D], preferred_element_type=f32)[0:8]
        b1 = b1_ref[...].astype(f32).reshape(1, F)
        b2 = b2_ref[...].astype(f32).reshape(1, D)

        def proj_ln(i, slot):
            rr = pl.multiple_of(i * r2, r2)
            attn = lax.dot_general(oT_s[:, pl.ds(rr, r2)], wo_ref[...], TN, preferred_element_type=f32)
            x1 = x_ref[pl.ds(rr, r2), :].astype(f32) + mod_s[0:1, 0:D] * attn
            x1_s[slot][...] = x1
            h = _ln(x1) * (1.0 + mod_s[0:1, 2 * D:3 * D]) + mod_s[0:1, D:2 * D]
            h2_s[slot][...] = h.astype(bf16)

        def out_copy(i):
            rr = pl.multiple_of(i * r2, r2)
            return pltpu.make_async_copy(out_s.at[pl.ds(rr, r2), :], o_hbm.at[pl.ds(rr, r2), :], osems.at[i])

        def ffn(i, slot, between):
            rr = pl.multiple_of(i * r2, r2)
            h1 = jnp.dot(h2_s[slot][...], w1_ref[...], preferred_element_type=f32) + b1
            h1 = jnp.maximum(h1, 0.0)
            h1 = (h1 * h1).astype(bf16)
            between()
            y = jnp.dot(h1, w2_ref[...], preferred_element_type=f32) + b2
            out_s[pl.ds(rr, r2), :] = (x1_s[slot][...] + mod_s[0:1, 3 * D:4 * D] * y).astype(out_s.dtype)
            out_copy(i).start()

        def tail(j, carry):
            i = 2 * j
            ffn(i, 0, lambda: proj_ln(i + 1, 1))
            ffn(i + 1, 1, lambda: proj_ln(jnp.minimum(i + 2, n2 - 1), 0))
            return carry
        proj_ln(0, 0)
        lax.fori_loop(0, n2 // 2, tail, 0)
        for i in range(n2):
            out_copy(i).wait()

    any_spec = pl.BlockSpec(memory_space=pl.ANY)
    return functools.partial(
        pl.pallas_call,
        kernel,
        in_specs=[any_spec] * 9,
        out_specs=any_spec,
        scratch_shapes=[
            pltpu.VMEM((S, D), bf16), pltpu.VMEM((D, 3 * D), bf16), pltpu.VMEM((D, D), bf16),
            pltpu.VMEM((D, F), bf16), pltpu.VMEM((F, D), bf16), pltpu.VMEM((D, 6 * D), bf16),
            pltpu.VMEM((8, 4 * D), f32), pltpu.VMEM((2 * D, D), bf16), pltpu.VMEM((D, S), bf16),
            pltpu.VMEM((S, D), bf16), pltpu.VMEM((D, S), bf16), pltpu.VMEM((H, S), f32),
            pltpu.VMEM((H, 128), f32), pltpu.VMEM((D, S), bf16), pltpu.VMEM((S, D), bf16),
            pltpu.VMEM((S, D), bf16), pltpu.VMEM((lag, kc, bq), f32), pltpu.VMEM((r2, D), f32),
            pltpu.VMEM((r2, D), f32), pltpu.VMEM((r2, D), bf16), pltpu.VMEM((r2, D), bf16),
            pltpu.VMEM((1, D), bf16), pltpu.VMEM((F,), bf16), pltpu.VMEM((D,), bf16),
            pltpu.SemaphoreType.DMA((11,)), pltpu.SemaphoreType.DMA((n1,)), pltpu.SemaphoreType.DMA((n2,)),
        ],
        compiler_params=pltpu.CompilerParams(vmem_limit_bytes=100 * 1024 * 1024),
        name="fused_adaln_block",
    )


def _build(**kw):
    def fn(A_x, A_wqkv, A_wo, B_x, B_w1, B_b1, B_w2, B_b2, c, w_mod):
        del B_x
        out = make_kernel(**kw)(out_shape=jax.ShapeDtypeStruct((S, D), A_x.dtype))(
            A_x.reshape(S, D), A_wqkv, A_wo, B_w1, B_b1, B_w2, B_b2, c, w_mod)
        return out.reshape(A_x.shape)
    return fn


@jax.jit
def pallas_adaLN_cond__mha_block__dense_activation_squared_relu__prompt_kernel(
    A_x: jax.Array,
    A_wqkv: jax.Array,
    A_wo: jax.Array,
    B_x: jax.Array,
    B_w1: jax.Array,
    B_b1: jax.Array,
    B_w2: jax.Array,
    B_b2: jax.Array,
    c: jax.Array,
    w_mod: jax.Array,
):
    return _build()(A_x, A_wqkv, A_wo, B_x, B_w1, B_b1, B_w2, B_b2, c, w_mod)
```

```python
import functools
import jax
import jax.numpy as jnp
from jax import lax
from jax.experimental import pallas as pl
from jax.experimental.pallas import tpu as pltpu

S, D, H, DH, F = 2048, 512, 32, 16, 1792
QSCALE = 0.25 * 1.4426950408889634
EPS = 1e-5
BOUND_SLACK = 1.01
L_MIN = float(2.0 ** -90)
NT = (((1,), (1,)), ((), ()))
TN = (((0,), (0,)), ((), ()))
f32 = jnp.float32
bf16 = jnp.bfloat16


def _ln(x):
    m = jnp.mean(x, axis=-1, keepdims=True)
    d = x - m
    v = jnp.mean(d * d, axis=-1, keepdims=True)
    return d * lax.rsqrt(v + EPS)


def make_kernel(bq=512, kc=128, lag=2, hu=16, r1=512, r2=128, lp=64, early=True, qvpu=True, kvpu=True):
    nq = S // bq
    nc = S // kc
    n1 = S // r1
    n2 = S // r2
    G = H // hu
    nit = nq * G

    def kernel(x_hbm, wqkv_hbm, wo_hbm, w1_hbm, b1_hbm, w2_hbm, b2_hbm, c_hbm, wmod_hbm,
               o_hbm,
               x_ref, wqkv_ref, wo_ref, w1_ref, w2_ref, wmod_ref,
               mod_s, wT_s, qT_s, k_s, vT_s, qn_s, kn_s, oT_s, out_s, h_s, sp_s, x1a_s, x1b_s, h2a_s, h2b_s,
               c_ref, b1_ref, b2_ref, sems, xsems, osems):
        x1_s = (x1a_s, x1b_s)
        h2_s = (h2a_s, h2b_s)

        def cols(hbm, vmem, start, size, sem):
            return pltpu.make_async_copy(hbm.at[:, pl.ds(start, size)], vmem.at[:, pl.ds(start, size)], sem)

        def x_copy(i):
            return pltpu.make_async_copy(x_hbm.at[pl.ds(i * r1, r1), :], x_ref.at[pl.ds(i * r1, r1), :], xsems.at[i])

        cp_mod1 = cols(wmod_hbm, wmod_ref, 0, 2 * D, sems.at[0])
        cp_wk = cols(wqkv_hbm, wqkv_ref, D, D, sems.at[1])
        cp_wq = cols(wqkv_hbm, wqkv_ref, 0, D, sems.at[2])
        cp_wv = cols(wqkv_hbm, wqkv_ref, 2 * D, D, sems.at[3])
        cp_mod2 = cols(wmod_hbm, wmod_ref, 2 * D, 4 * D, sems.at[4])
        cp_wo = pltpu.make_async_copy(wo_hbm, wo_ref, sems.at[5])
        cp_w1 = pltpu.make_async_copy(w1_hbm, w1_ref, sems.at[6])
        cp_w2 = pltpu.make_async_copy(w2_hbm, w2_ref, sems.at[7])
        cp_c = pltpu.make_async_copy(c_hbm, c_ref, sems.at[8])
        cp_b1 = pltpu.make_async_copy(b1_hbm, b1_ref, sems.at[9])
        cp_b2 = pltpu.make_async_copy(b2_hbm, b2_ref, sems.at[10])
        cp_c.start()
        cp_mod1.start()
        x_copy(0).start()
        cp_wk.start()
        cp_wq.start()

        cp_c.wait()
        c = c_ref[...].astype(f32)
        sc = jnp.broadcast_to(c * jax.nn.sigmoid(c), (16, D)).astype(bf16)
        cp_mod1.wait()
        mod1 = jnp.dot(sc, wmod_ref[:, 0:2 * D], preferred_element_type=f32)
        sa = mod1[0:1, 0:D]
        ca1 = 1.0 + mod1[0:1, D:2 * D]

        def ln_rows(r, n):
            x = x_ref[r:r + n, :].astype(f32)
            h_s[r:r + n, :] = (_ln(x) * ca1 + sa).astype(bf16)

        ehead = (lax.broadcasted_iota(jnp.int32, (H, D), 1) // DH
                 == lax.broadcasted_iota(jnp.int32, (H, D), 0)).astype(bf16)

        def k_rows(r, n):
            k = jnp.dot(h_s[pl.ds(r, n), :], wqkv_ref[:, D:2 * D], preferred_element_type=f32)
            k_s[pl.ds(r, n), :] = k.astype(bf16)
            return k

        def k_norm(k):
            return lax.dot_general(ehead, (k * k).astype(bf16), NT, preferred_element_type=f32)

        def q_cols(r, n):
            qT = lax.dot_general(wT_s[0:D, :], h_s[pl.ds(r, n), :], NT, preferred_element_type=f32) * QSCALE
            qT_s[:, pl.ds(r, n)] = qT.astype(bf16)
            if qvpu:
                qn2 = jnp.sum((qT * qT).reshape(H, DH, n), axis=1)
            else:
                qn2 = jnp.dot(ehead, (qT * qT).astype(bf16), preferred_element_type=f32)
            qn_s[:, pl.ds(r, n)] = jnp.sqrt(qn2)

        def v_cols(r, n):
            vT = lax.dot_general(wT_s[D:2 * D, :], h_s[pl.ds(r, n), :], NT, preferred_element_type=f32)
            vT_s[:, pl.ds(r, n)] = vT.astype(bf16)

        x_copy(0).wait()
        ln_rows(0, r1)
        cp_wk.wait()
        x_copy(1).start()
        cp_wv.start()
        for i in range(2, n1):
            x_copy(i).start()
        ka = k_rows(0, r1 // 2)
        cp_wq.wait()
        wT_s[0:D, :] = wqkv_ref[:, 0:D].T
        kb = k_rows(r1 // 2, r1 // 2)
        kmax = k_norm(jnp.concatenate([ka, kb], axis=0))
        qr = r1 // 4
        cp_wv.wait()
        x_copy(1).wait()
        for t in range(4):
            q_cols(t * qr, qr)
            if t == 0:
                wT_s[D:2 * D, :] = wqkv_ref[:, 2 * D:3 * D].T
            if t == 2 and kvpu:
                wT_s[2 * D:3 * D, :] = wqkv_ref[:, D:2 * D].T
            for z in range(qr // lp):
                ln_rows(r1 + t * qr + z * lp, lp)
        for i in range(2, n1):
            x_copy(i).wait()
        cp_mod2.start()
        cp_wo.start()
        cp_b1.start()
        cp_b2.start()
        cp_w1.start()
        cp_w2.start()
        for t in range(4):
            v_cols(t * qr, qr)
            for z in range(2 * qr // lp):
                ln_rows(2 * r1 + t * 2 * qr + z * lp, lp)

        def rows(i, kmax):
            rr = pl.multiple_of(i * r1, r1)
            if kvpu:
                kT = lax.dot_general(wT_s[2 * D:3 * D, :], h_s[pl.ds(rr, r1), :], NT, preferred_element_type=f32)
                k_s[pl.ds(rr, r1), :] = kT.astype(bf16).T
                kmax = jnp.maximum(kmax, jnp.sum((kT * kT).reshape(H, DH, r1), axis=1))
            else:
                kmax = jnp.maximum(kmax, k_norm(k_rows(rr, r1)))
            q_cols(rr, r1)
            v_cols(rr, r1)
            return kmax
        kmax = lax.fori_loop(1, n1, rows, kmax)
        kn_s[...] = jnp.broadcast_to(jnp.sqrt(jnp.max(kmax, axis=1, keepdims=True)) * BOUND_SLACK, (H, 128))

        def pv_stage(s, d, cc):
            p = jnp.exp2(s.reshape(kc // 8, 8, bq) - d['m'][None])
            ls = jnp.sum(p, axis=0)
            d['l'] = ls if d['l'] is None else d['l'] + ls
            r = jnp.dot(vT_s[pl.ds(d['hoff'], DH), cc * kc:(cc + 1) * kc], p.reshape(kc, bq).astype(bf16),
                        preferred_element_type=f32)
            d['acc'] = r if d['acc'] is None else d['acc'] + r

        def finalize(d, lmin):
            lsum = jnp.sum(d['l'], axis=0, keepdims=True)
            oT_s[pl.ds(d['hoff'], DH), pl.ds(d['q0'], bq)] = (d['acc'] * (1.0 / lsum)).astype(bf16)
            return jnp.minimum(lmin, lsum)

        def prev_state(itp, l, acc, m):
            hp = (itp % G) * hu + (hu - 1)
            return dict(hoff=pl.multiple_of(hp * DH, DH), q0=pl.multiple_of((itp // G) * bq, bq), l=l, acc=acc, m=m)

        def heads(it, carry):
            lmin, l_p, acc_p, m_p = carry
            prev = prev_state((it + nit - 1) % nit, l_p, acc_p, m_p)
            hg = it % G
            q0 = pl.multiple_of((it // G) * bq, bq)
            items = []
            st = {}
            for u in range(hu):
                h = hg * hu + u
                goff = pl.multiple_of((hg * hu + u) // 8 * 128, 128)
                hoff = pl.multiple_of(h * DH, DH)
                jj = u % 8
                parts = [qT_s[pl.ds(hoff, DH), pl.ds(q0, bq)]]
                if jj > 0:
                    parts.insert(0, jnp.zeros((DH * jj, bq), bf16))
                if jj < 7:
                    parts.append(jnp.zeros((DH * (7 - jj), bq), bf16))
                qm = jnp.concatenate(parts, axis=0)
                kn = jnp.concatenate([kn_s[pl.ds(h, 1), :]] * (bq // 128), axis=1)
                m = jnp.broadcast_to(qn_s[pl.ds(h, 1), pl.ds(q0, bq)] * kn, (8, bq))
                st[u] = dict(goff=goff, hoff=hoff, q0=q0, qm=qm, m=m, l=None, acc=None)
                for cc in range(nc):
                    items.append((u, cc))
            svals = {}
            n = len(items)
            for t in range(n):
                u, cc = items[t]
                d = st[u]
                svals[t] = jnp.dot(k_s[cc * kc:(cc + 1) * kc, pl.ds(d['goff'], 128)], d['qm'],
                                   preferred_element_type=f32)
                if t < lag:
                    pv_stage(sp_s[t], prev, nc - lag + t)
                    if t == lag - 1:
                        lmin = finalize(prev, lmin)
                else:
                    u, cc = items[t - lag]
                    pv_stage(svals.pop(t - lag), st[u], cc)
                    if cc == nc - 1:
                        lmin = finalize(st[u], lmin)
            for t in range(lag):
                sp_s[t] = svals.pop(n - lag + t)
            d = st[hu - 1]
            return lmin, d['l'], d['acc'], d['m']

        sp_s[...] = jnp.zeros(sp_s.shape, f32)
        init = (jnp.full((1, bq), 1.0, f32), jnp.zeros((8, bq), f32), jnp.zeros((DH, bq), f32),
                jnp.zeros((8, bq), f32))
        lmin, l_p, acc_p, m_p = lax.fori_loop(0, nit, heads, init)
        cp_mod2.wait()
        cp_wo.wait()
        cp_b1.wait()
        cp_b2.wait()
        cp_w1.wait()
        cp_w2.wait()

        def proj_ln(i, slot):
            rr = pl.multiple_of(i * r2, r2)
            attn = lax.dot_general(oT_s[:, pl.ds(rr, r2)], wo_ref[...], TN, preferred_element_type=f32)
            x1 = x_ref[pl.ds(rr, r2), :].astype(f32) + mod_s[0:1, 0:D] * attn
            x1_s[slot][...] = x1
            h = _ln(x1) * (1.0 + mod_s[0:1, 2 * D:3 * D]) + mod_s[0:1, D:2 * D]
            h2_s[slot][...] = h.astype(bf16)

        last = prev_state(nit - 1, l_p, acc_p, m_p)
        for t in range(lag):
            pv_stage(sp_s[t], last, nc - lag + t)
        lmin = finalize(last, lmin)
        if early:
            mod_s[...] = jnp.dot(sc, wmod_ref[:, 2 * D:6 * D], preferred_element_type=f32)[0:8]
            proj_ln(0, 0)
        unsafe = jnp.logical_not(jnp.min(lmin) >= L_MIN)

        @pl.when(unsafe)
        def _():
            row_f = lax.broadcasted_iota(jnp.int32, (128, 128), 0)

            def one(it, carry):
                h = it % H
                q0 = pl.multiple_of((it // H) * 128, 128)
                goff = pl.multiple_of(h // 8 * 128, 128)
                hoff = pl.multiple_of(h * DH, DH)
                qg = qT_s[pl.ds(goff, 128), pl.ds(q0, 128)]
                qm = jnp.where(row_f // DH == h % 8, qg, jnp.zeros_like(qg))
                s = jnp.dot(k_s[:, pl.ds(goff, 128)], qm, preferred_element_type=f32)
                p = jnp.exp2(s - jnp.max(s, axis=0, keepdims=True))
                l = jnp.sum(p, axis=0, keepdims=True)
                o = jnp.dot(vT_s[pl.ds(hoff, DH), :], p.astype(bf16), preferred_element_type=f32)
                oT_s[pl.ds(hoff, DH), pl.ds(q0, 128)] = (o / l).astype(bf16)
                return carry
            lax.fori_loop(0, (S // 128) * H, one, 0)
            if early:
                proj_ln(0, 0)

        if not early:
            mod_s[...] = jnp.dot(sc, wmod_ref[:, 2 * D:6 * D], preferred_element_type=f32)[0:8]
        b1 = b1_ref[...].astype(f32).reshape(1, F)
        b2 = b2_ref[...].astype(f32).reshape(1, D)

        def out_copy(i):
            rr = pl.multiple_of(i * r2, r2)
            return pltpu.make_async_copy(out_s.at[pl.ds(rr, r2), :], o_hbm.at[pl.ds(rr, r2), :], osems.at[i])

        def ffn(i, slot, between):
            rr = pl.multiple_of(i * r2, r2)
            h1 = jnp.dot(h2_s[slot][...], w1_ref[...], preferred_element_type=f32) + b1
            h1 = jnp.maximum(h1, 0.0)
            h1 = (h1 * h1).astype(bf16)
            between()
            y = jnp.dot(h1, w2_ref[...], preferred_element_type=f32) + b2
            out_s[pl.ds(rr, r2), :] = (x1_s[slot][...] + mod_s[0:1, 3 * D:4 * D] * y).astype(out_s.dtype)
            out_copy(i).start()

        def tail(j, carry):
            i = 2 * j
            ffn(i, 0, lambda: proj_ln(i + 1, 1))
            ffn(i + 1, 1, lambda: proj_ln(jnp.minimum(i + 2, n2 - 1), 0))
            return carry
        if not early:
            proj_ln(0, 0)
        lax.fori_loop(0, n2 // 2, tail, 0)
        for i in range(n2):
            out_copy(i).wait()

    any_spec = pl.BlockSpec(memory_space=pl.ANY)
    return functools.partial(
        pl.pallas_call,
        kernel,
        in_specs=[any_spec] * 9,
        out_specs=any_spec,
        scratch_shapes=[
            pltpu.VMEM((S, D), bf16), pltpu.VMEM((D, 3 * D), bf16), pltpu.VMEM((D, D), bf16),
            pltpu.VMEM((D, F), bf16), pltpu.VMEM((F, D), bf16), pltpu.VMEM((D, 6 * D), bf16),
            pltpu.VMEM((8, 4 * D), f32), pltpu.VMEM((3 * D, D), bf16), pltpu.VMEM((D, S), bf16),
            pltpu.VMEM((S, D), bf16), pltpu.VMEM((D, S), bf16), pltpu.VMEM((H, S), f32),
            pltpu.VMEM((H, 128), f32), pltpu.VMEM((D, S), bf16), pltpu.VMEM((S, D), bf16),
            pltpu.VMEM((S, D), bf16), pltpu.VMEM((lag, kc, bq), f32), pltpu.VMEM((r2, D), f32),
            pltpu.VMEM((r2, D), f32), pltpu.VMEM((r2, D), bf16), pltpu.VMEM((r2, D), bf16),
            pltpu.VMEM((1, D), bf16), pltpu.VMEM((F,), bf16), pltpu.VMEM((D,), bf16),
            pltpu.SemaphoreType.DMA((11,)), pltpu.SemaphoreType.DMA((n1,)), pltpu.SemaphoreType.DMA((n2,)),
        ],
        compiler_params=pltpu.CompilerParams(vmem_limit_bytes=100 * 1024 * 1024),
        name="fused_adaln_block",
    )


def _build(**kw):
    def fn(A_x, A_wqkv, A_wo, B_x, B_w1, B_b1, B_w2, B_b2, c, w_mod):
        del B_x
        out = make_kernel(**kw)(out_shape=jax.ShapeDtypeStruct((S, D), A_x.dtype))(
            A_x.reshape(S, D), A_wqkv, A_wo, B_w1, B_b1, B_w2, B_b2, c, w_mod)
        return out.reshape(A_x.shape)
    return fn


@jax.jit
def pallas_adaLN_cond__mha_block__dense_activation_squared_relu__prompt_kernel(
    A_x: jax.Array,
    A_wqkv: jax.Array,
    A_wo: jax.Array,
    B_x: jax.Array,
    B_w1: jax.Array,
    B_b1: jax.Array,
    B_w2: jax.Array,
    B_b2: jax.Array,
    c: jax.Array,
    w_mod: jax.Array,
):
    return _build()(A_x, A_wqkv, A_wo, B_x, B_w1, B_b1, B_w2, B_b2, c, w_mod)
```

```python
import functools
import jax
import jax.numpy as jnp
from jax import lax
from jax.experimental import pallas as pl
from jax.experimental.pallas import tpu as pltpu

S, D, H, DH, F = 2048, 512, 32, 16, 1792
QSCALE = 0.25 * 1.4426950408889634
EPS = 1e-5
BOUND_SLACK = 1.01
L_MIN = float(2.0 ** -90)
NT = (((1,), (1,)), ((), ()))
TN = (((0,), (0,)), ((), ()))
f32 = jnp.float32
bf16 = jnp.bfloat16


def _ln(x):
    m = jnp.mean(x, axis=-1, keepdims=True)
    d = x - m
    v = jnp.mean(d * d, axis=-1, keepdims=True)
    return d * lax.rsqrt(v + EPS)


def make_kernel(bq=512, kc=128, lag=2, hu=16, r1=512, r2=128, lp=64):
    nq = S // bq
    nc = S // kc
    n1 = S // r1
    n2 = S // r2
    G = H // hu
    nit = nq * G

    def kernel(x_hbm, wqkv_hbm, wo_hbm, w1_hbm, b1_hbm, w2_hbm, b2_hbm, c_hbm, wmod_hbm,
               o_hbm,
               x_ref, wqkv_ref, wo_ref, w1_ref, w2_ref, wmod_ref,
               mod_s, wT_s, qT_s, k_s, vT_s, qn_s, kn_s, oT_s, out_s, h_s, sp_s, x1a_s, x1b_s, h2a_s, h2b_s,
               c_ref, b1_ref, b2_ref, sems, xsems, osems):
        x1_s = (x1a_s, x1b_s)
        h2_s = (h2a_s, h2b_s)

        def cols(hbm, vmem, start, size, sem):
            return pltpu.make_async_copy(hbm.at[:, pl.ds(start, size)], vmem.at[:, pl.ds(start, size)], sem)

        def x_copy(i):
            return pltpu.make_async_copy(x_hbm.at[pl.ds(i * r1, r1), :], x_ref.at[pl.ds(i * r1, r1), :], xsems.at[i])

        cp_mod1 = cols(wmod_hbm, wmod_ref, 0, 2 * D, sems.at[0])
        cp_wk = cols(wqkv_hbm, wqkv_ref, D, D, sems.at[1])
        cp_wq = cols(wqkv_hbm, wqkv_ref, 0, D, sems.at[2])
        cp_wv = cols(wqkv_hbm, wqkv_ref, 2 * D, D, sems.at[3])
        cp_mod2 = cols(wmod_hbm, wmod_ref, 2 * D, 4 * D, sems.at[4])
        cp_wo = pltpu.make_async_copy(wo_hbm, wo_ref, sems.at[5])
        cp_w1 = pltpu.make_async_copy(w1_hbm, w1_ref, sems.at[6])
        cp_w2 = pltpu.make_async_copy(w2_hbm, w2_ref, sems.at[7])
        cp_c = pltpu.make_async_copy(c_hbm, c_ref, sems.at[8])
        cp_b1 = pltpu.make_async_copy(b1_hbm, b1_ref, sems.at[9])
        cp_b2 = pltpu.make_async_copy(b2_hbm, b2_ref, sems.at[10])
        cp_c.start()
        hr = r1 // 2
        cp_x0a = pltpu.make_async_copy(x_hbm.at[pl.ds(0, hr), :], x_ref.at[pl.ds(0, hr), :], sems.at[11])
        cp_x0b = pltpu.make_async_copy(x_hbm.at[pl.ds(hr, hr), :], x_ref.at[pl.ds(hr, hr), :], xsems.at[0])
        cp_mod1.start()
        cp_x0a.start()
        cp_wk.start()
        cp_x0b.start()
        cp_wq.start()

        cp_c.wait()
        c = c_ref[...].astype(f32)
        sc = jnp.broadcast_to(c * jax.nn.sigmoid(c), (16, D)).astype(bf16)
        cp_mod1.wait()
        mod1 = jnp.dot(sc, wmod_ref[:, 0:2 * D], preferred_element_type=f32)
        sa = mod1[0:1, 0:D]
        ca1 = 1.0 + mod1[0:1, D:2 * D]

        def ln_rows(r, n):
            x = x_ref[r:r + n, :].astype(f32)
            h_s[r:r + n, :] = (_ln(x) * ca1 + sa).astype(bf16)

        ehead = (lax.broadcasted_iota(jnp.int32, (H, D), 1) // DH
                 == lax.broadcasted_iota(jnp.int32, (H, D), 0)).astype(bf16)

        def k_rows(r, n):
            k = jnp.dot(h_s[pl.ds(r, n), :], wqkv_ref[:, D:2 * D], preferred_element_type=f32)
            k_s[pl.ds(r, n), :] = k.astype(bf16)
            return k

        def k_norm(k):
            return lax.dot_general(ehead, (k * k).astype(bf16), NT, preferred_element_type=f32)

        def q_cols(r, n):
            qT = lax.dot_general(wT_s[0:D, :], h_s[pl.ds(r, n), :], NT, preferred_element_type=f32) * QSCALE
            qT_s[:, pl.ds(r, n)] = qT.astype(bf16)
            qn_s[:, pl.ds(r, n)] = jnp.sqrt(jnp.sum((qT * qT).reshape(H, DH, n), axis=1))

        def v_cols(r, n):
            vT = lax.dot_general(wT_s[D:2 * D, :], h_s[pl.ds(r, n), :], NT, preferred_element_type=f32)
            vT_s[:, pl.ds(r, n)] = vT.astype(bf16)

        cp_x0a.wait()
        ln_rows(0, hr)
        cp_wk.wait()
        cp_x0b.wait()
        x_copy(1).start()
        cp_wv.start()
        for i in range(2, n1):
            x_copy(i).start()
        ka = k_rows(0, hr)
        ln_rows(hr, hr)
        cp_wq.wait()
        wT_s[0:D, :] = wqkv_ref[:, 0:D].T
        kb = k_rows(hr, hr)
        kmax = k_norm(jnp.concatenate([ka, kb], axis=0))
        qr = r1 // 4
        cp_wv.wait()
        x_copy(1).wait()
        for t in range(4):
            q_cols(t * qr, qr)
            if t == 0:
                wT_s[D:2 * D, :] = wqkv_ref[:, 2 * D:3 * D].T
            if t == 2:
                wT_s[2 * D:3 * D, :] = wqkv_ref[:, D:2 * D].T
            for z in range(qr // lp):
                ln_rows(r1 + t * qr + z * lp, lp)
        for i in range(2, n1):
            x_copy(i).wait()
        cp_mod2.start()
        cp_wo.start()
        cp_b1.start()
        cp_b2.start()
        cp_w1.start()
        cp_w2.start()
        for t in range(4):
            v_cols(t * qr, qr)
            for z in range(2 * qr // lp):
                ln_rows(2 * r1 + t * 2 * qr + z * lp, lp)

        def rows(i, kmax):
            rr = pl.multiple_of(i * r1, r1)
            kT = lax.dot_general(wT_s[2 * D:3 * D, :], h_s[pl.ds(rr, r1), :], NT, preferred_element_type=f32)
            k_s[pl.ds(rr, r1), :] = kT.astype(bf16).T
            kmax = jnp.maximum(kmax, jnp.sum((kT * kT).reshape(H, DH, r1), axis=1))
            q_cols(rr, r1)
            v_cols(rr, r1)
            return kmax
        kmax = lax.fori_loop(1, n1, rows, kmax)
        kn_s[...] = jnp.broadcast_to(jnp.sqrt(jnp.max(kmax, axis=1, keepdims=True)) * BOUND_SLACK, (H, 128))

        def pv_stage(s, d, cc):
            p = jnp.exp2(s.reshape(kc // 8, 8, bq) - d['m'][None])
            ls = jnp.sum(p, axis=0)
            d['l'] = ls if d['l'] is None else d['l'] + ls
            r = jnp.dot(vT_s[pl.ds(d['hoff'], DH), cc * kc:(cc + 1) * kc], p.reshape(kc, bq).astype(bf16),
                        preferred_element_type=f32)
            d['acc'] = r if d['acc'] is None else d['acc'] + r

        def finalize(d, lmin):
            lsum = jnp.sum(d['l'], axis=0, keepdims=True)
            oT_s[pl.ds(d['hoff'], DH), pl.ds(d['q0'], bq)] = (d['acc'] * (1.0 / lsum)).astype(bf16)
            return jnp.minimum(lmin, lsum)

        def prev_state(itp, l, acc, m):
            hp = (itp % G) * hu + (hu - 1)
            return dict(hoff=pl.multiple_of(hp * DH, DH), q0=pl.multiple_of((itp // G) * bq, bq), l=l, acc=acc, m=m)

        def heads(it, carry):
            lmin, l_p, acc_p, m_p = carry
            prev = prev_state((it + nit - 1) % nit, l_p, acc_p, m_p)
            hg = it % G
            q0 = pl.multiple_of((it // G) * bq, bq)
            items = []
            st = {}
            for u in range(hu):
                h = hg * hu + u
                goff = pl.multiple_of((hg * hu + u) // 8 * 128, 128)
                hoff = pl.multiple_of(h * DH, DH)
                jj = u % 8
                parts = [qT_s[pl.ds(hoff, DH), pl.ds(q0, bq)]]
                if jj > 0:
                    parts.insert(0, jnp.zeros((DH * jj, bq), bf16))
                if jj < 7:
                    parts.append(jnp.zeros((DH * (7 - jj), bq), bf16))
                qm = jnp.concatenate(parts, axis=0)
                kn = jnp.concatenate([kn_s[pl.ds(h, 1), :]] * (bq // 128), axis=1)
                m = jnp.broadcast_to(qn_s[pl.ds(h, 1), pl.ds(q0, bq)] * kn, (8, bq))
                st[u] = dict(goff=goff, hoff=hoff, q0=q0, qm=qm, m=m, l=None, acc=None)
                for cc in range(nc):
                    items.append((u, cc))
            svals = {}
            n = len(items)
            for t in range(n):
                u, cc = items[t]
                d = st[u]
                svals[t] = jnp.dot(k_s[cc * kc:(cc + 1) * kc, pl.ds(d['goff'], 128)], d['qm'],
                                   preferred_element_type=f32)
                if t < lag:
                    pv_stage(sp_s[t], prev, nc - lag + t)
                    if t == lag - 1:
                        lmin = finalize(prev, lmin)
                else:
                    u, cc = items[t - lag]
                    pv_stage(svals.pop(t - lag), st[u], cc)
                    if cc == nc - 1:
                        lmin = finalize(st[u], lmin)
            for t in range(lag):
                sp_s[t] = svals.pop(n - lag + t)
            d = st[hu - 1]
            return lmin, d['l'], d['acc'], d['m']

        sp_s[...] = jnp.zeros(sp_s.shape, f32)
        init = (jnp.full((1, bq), 1.0, f32), jnp.zeros((8, bq), f32), jnp.zeros((DH, bq), f32),
                jnp.zeros((8, bq), f32))
        lmin, l_p, acc_p, m_p = lax.fori_loop(0, nit, heads, init)
        cp_mod2.wait()
        cp_wo.wait()
        cp_b1.wait()
        cp_b2.wait()
        cp_w1.wait()
        cp_w2.wait()

        def proj_ln(i, slot):
            rr = pl.multiple_of(i * r2, r2)
            attn = lax.dot_general(oT_s[:, pl.ds(rr, r2)], wo_ref[...], TN, preferred_element_type=f32)
            x1 = x_ref[pl.ds(rr, r2), :].astype(f32) + mod_s[0:1, 0:D] * attn
            x1_s[slot][...] = x1
            h = _ln(x1) * (1.0 + mod_s[0:1, 2 * D:3 * D]) + mod_s[0:1, D:2 * D]
            h2_s[slot][...] = h.astype(bf16)

        last = prev_state(nit - 1, l_p, acc_p, m_p)
        for t in range(lag):
            pv_stage(sp_s[t], last, nc - lag + t)
        lmin = finalize(last, lmin)
        mod_s[...] = jnp.dot(sc, wmod_ref[:, 2 * D:6 * D], preferred_element_type=f32)[0:8]
        proj_ln(0, 0)
        unsafe = jnp.logical_not(jnp.min(lmin) >= L_MIN)

        @pl.when(unsafe)
        def _():
            row_f = lax.broadcasted_iota(jnp.int32, (128, 128), 0)

            def one(it, carry):
                h = it % H
                q0 = pl.multiple_of((it // H) * 128, 128)
                goff = pl.multiple_of(h // 8 * 128, 128)
                hoff = pl.multiple_of(h * DH, DH)
                qg = qT_s[pl.ds(goff, 128), pl.ds(q0, 128)]
                qm = jnp.where(row_f // DH == h % 8, qg, jnp.zeros_like(qg))
                s = jnp.dot(k_s[:, pl.ds(goff, 128)], qm, preferred_element_type=f32)
                p = jnp.exp2(s - jnp.max(s, axis=0, keepdims=True))
                l = jnp.sum(p, axis=0, keepdims=True)
                o = jnp.dot(vT_s[pl.ds(hoff, DH), :], p.astype(bf16), preferred_element_type=f32)
                oT_s[pl.ds(hoff, DH), pl.ds(q0, 128)] = (o / l).astype(bf16)
                return carry
            lax.fori_loop(0, (S // 128) * H, one, 0)
            proj_ln(0, 0)

        b1 = b1_ref[...].astype(f32).reshape(1, F)
        b2 = b2_ref[...].astype(f32).reshape(1, D)

        def out_copy(i):
            rr = pl.multiple_of(i * r2, r2)
            return pltpu.make_async_copy(out_s.at[pl.ds(rr, r2), :], o_hbm.at[pl.ds(rr, r2), :], osems.at[i])

        def ffn(i, slot, between):
            rr = pl.multiple_of(i * r2, r2)
            h1 = jnp.dot(h2_s[slot][...], w1_ref[...], preferred_element_type=f32) + b1
            h1 = jnp.maximum(h1, 0.0)
            h1 = (h1 * h1).astype(bf16)
            between()
            y = jnp.dot(h1, w2_ref[...], preferred_element_type=f32) + b2
            out_s[pl.ds(rr, r2), :] = (x1_s[slot][...] + mod_s[0:1, 3 * D:4 * D] * y).astype(out_s.dtype)
            out_copy(i).start()

        def tail(j, carry):
            i = 2 * j
            ffn(i, 0, lambda: proj_ln(i + 1, 1))
            ffn(i + 1, 1, lambda: proj_ln(jnp.minimum(i + 2, n2 - 1), 0))
            return carry
        lax.fori_loop(0, n2 // 2, tail, 0)
        for i in range(n2):
            out_copy(i).wait()

    any_spec = pl.BlockSpec(memory_space=pl.ANY)
    return functools.partial(
        pl.pallas_call,
        kernel,
        in_specs=[any_spec] * 9,
        out_specs=any_spec,
        scratch_shapes=[
            pltpu.VMEM((S, D), bf16), pltpu.VMEM((D, 3 * D), bf16), pltpu.VMEM((D, D), bf16),
            pltpu.VMEM((D, F), bf16), pltpu.VMEM((F, D), bf16), pltpu.VMEM((D, 6 * D), bf16),
            pltpu.VMEM((8, 4 * D), f32), pltpu.VMEM((3 * D, D), bf16), pltpu.VMEM((D, S), bf16),
            pltpu.VMEM((S, D), bf16), pltpu.VMEM((D, S), bf16), pltpu.VMEM((H, S), f32),
            pltpu.VMEM((H, 128), f32), pltpu.VMEM((D, S), bf16), pltpu.VMEM((S, D), bf16),
            pltpu.VMEM((S, D), bf16), pltpu.VMEM((lag, kc, bq), f32), pltpu.VMEM((r2, D), f32),
            pltpu.VMEM((r2, D), f32), pltpu.VMEM((r2, D), bf16), pltpu.VMEM((r2, D), bf16),
            pltpu.VMEM((1, D), bf16), pltpu.VMEM((F,), bf16), pltpu.VMEM((D,), bf16),
            pltpu.SemaphoreType.DMA((12,)), pltpu.SemaphoreType.DMA((n1,)), pltpu.SemaphoreType.DMA((n2,)),
        ],
        compiler_params=pltpu.CompilerParams(vmem_limit_bytes=100 * 1024 * 1024),
        name="fused_adaln_block",
    )


def _build(**kw):
    def fn(A_x, A_wqkv, A_wo, B_x, B_w1, B_b1, B_w2, B_b2, c, w_mod):
        del B_x
        out = make_kernel(**kw)(out_shape=jax.ShapeDtypeStruct((S, D), A_x.dtype))(
            A_x.reshape(S, D), A_wqkv, A_wo, B_w1, B_b1, B_w2, B_b2, c, w_mod)
        return out.reshape(A_x.shape)
    return fn


@jax.jit
def pallas_adaLN_cond__mha_block__dense_activation_squared_relu__prompt_kernel(
    A_x: jax.Array,
    A_wqkv: jax.Array,
    A_wo: jax.Array,
    B_x: jax.Array,
    B_w1: jax.Array,
    B_b1: jax.Array,
    B_w2: jax.Array,
    B_b2: jax.Array,
    c: jax.Array,
    w_mod: jax.Array,
):
    return _build()(A_x, A_wqkv, A_wo, B_x, B_w1, B_b1, B_w2, B_b2, c, w_mod)
```

```python
import functools
import jax
import jax.numpy as jnp
from jax import lax
from jax.experimental import pallas as pl
from jax.experimental.pallas import tpu as pltpu

S, D, H, DH, F = 2048, 512, 32, 16, 1792
QSCALE = 0.25 * 1.4426950408889634
EPS = 1e-5
BOUND_SLACK = 1.01
L_MIN = float(2.0 ** -90)
NT = (((1,), (1,)), ((), ()))
TN = (((0,), (0,)), ((), ()))
f32 = jnp.float32
bf16 = jnp.bfloat16


def _ln(x):
    m = jnp.mean(x, axis=-1, keepdims=True)
    d = x - m
    v = jnp.mean(d * d, axis=-1, keepdims=True)
    return d * lax.rsqrt(v + EPS)


def make_kernel(bq=512, kc=128, lag=2, hu=16, r1=512, r2=128, lp=64):
    nq = S // bq
    nc = S // kc
    n1 = S // r1
    n2 = S // r2
    G = H // hu
    nit = nq * G

    def kernel(x_hbm, wqkv_hbm, wo_hbm, w1_hbm, b1_hbm, w2_hbm, b2_hbm, c_hbm, wmod_hbm,
               o_hbm,
               x_ref, wqkv_ref, wo_ref, w1_ref, w2_ref, wmod_ref,
               mod_s, wT_s, qT_s, k_s, vT_s, qn_s, kn_s, oT_s, out_s, h_s, sp_s, x1a_s, x1b_s, h2a_s, h2b_s,
               c_ref, b1_ref, b2_ref, sems, xsems, osems):
        x1_s = (x1a_s, x1b_s)
        h2_s = (h2a_s, h2b_s)

        def cols(hbm, vmem, start, size, sem):
            return pltpu.make_async_copy(hbm.at[:, pl.ds(start, size)], vmem.at[:, pl.ds(start, size)], sem)

        def x_copy(i):
            return pltpu.make_async_copy(x_hbm.at[pl.ds(i * r1, r1), :], x_ref.at[pl.ds(i * r1, r1), :], xsems.at[i])

        cp_mod1 = cols(wmod_hbm, wmod_ref, 0, 2 * D, sems.at[0])
        cp_wk = cols(wqkv_hbm, wqkv_ref, D, D, sems.at[1])
        cp_wq = cols(wqkv_hbm, wqkv_ref, 0, D, sems.at[2])
        cp_wv = cols(wqkv_hbm, wqkv_ref, 2 * D, D, sems.at[3])
        cp_mod2 = cols(wmod_hbm, wmod_ref, 2 * D, 4 * D, sems.at[4])
        cp_wo = pltpu.make_async_copy(wo_hbm, wo_ref, sems.at[5])
        cp_w1 = pltpu.make_async_copy(w1_hbm, w1_ref, sems.at[6])
        cp_w2 = pltpu.make_async_copy(w2_hbm, w2_ref, sems.at[7])
        cp_c = pltpu.make_async_copy(c_hbm, c_ref, sems.at[8])
        cp_b1 = pltpu.make_async_copy(b1_hbm, b1_ref, sems.at[9])
        cp_b2 = pltpu.make_async_copy(b2_hbm, b2_ref, sems.at[10])
        cp_c.start()
        hr = r1 // 2
        cp_x0a = pltpu.make_async_copy(x_hbm.at[pl.ds(0, hr), :], x_ref.at[pl.ds(0, hr), :], sems.at[11])
        cp_x0b = pltpu.make_async_copy(x_hbm.at[pl.ds(hr, hr), :], x_ref.at[pl.ds(hr, hr), :], xsems.at[0])
        cp_mod1.start()
        cp_x0a.start()
        cp_wk.start()
        cp_x0b.start()
        cp_wq.start()

        cp_c.wait()
        c = c_ref[...].astype(f32)
        sc = jnp.broadcast_to(c * jax.nn.sigmoid(c), (16, D)).astype(bf16)
        cp_mod1.wait()
        mod1 = jnp.dot(sc, wmod_ref[:, 0:2 * D], preferred_element_type=f32)
        sa = mod1[0:1, 0:D]
        ca1 = 1.0 + mod1[0:1, D:2 * D]

        def ln_rows(r, n):
            x = x_ref[r:r + n, :].astype(f32)
            h_s[r:r + n, :] = (_ln(x) * ca1 + sa).astype(bf16)

        ehead = (lax.broadcasted_iota(jnp.int32, (H, D), 1) // DH
                 == lax.broadcasted_iota(jnp.int32, (H, D), 0)).astype(bf16)

        def k_rows(r, n):
            k = jnp.dot(h_s[pl.ds(r, n), :], wqkv_ref[:, D:2 * D], preferred_element_type=f32)
            k_s[pl.ds(r, n), :] = k.astype(bf16)
            return k

        def k_norm(k):
            return lax.dot_general(ehead, (k * k).astype(bf16), NT, preferred_element_type=f32)

        def q_cols(r, n):
            qT = lax.dot_general(wT_s[0:D, :], h_s[pl.ds(r, n), :], NT, preferred_element_type=f32) * QSCALE
            qT_s[:, pl.ds(r, n)] = qT.astype(bf16)
            qn_s[:, pl.ds(r, n)] = jnp.sqrt(jnp.sum((qT * qT).reshape(H, DH, n), axis=1))

        def v_cols(r, n):
            vT = lax.dot_general(wT_s[D:2 * D, :], h_s[pl.ds(r, n), :], NT, preferred_element_type=f32)
            vT_s[:, pl.ds(r, n)] = vT.astype(bf16)

        cp_x0a.wait()
        ln_rows(0, hr)
        cp_wk.wait()
        cp_x0b.wait()
        x_copy(1).start()
        cp_wv.start()
        for i in range(2, n1):
            x_copy(i).start()
        ka = k_rows(0, hr)
        ln_rows(hr, hr)
        cp_wq.wait()
        wT_s[0:D, :] = wqkv_ref[:, 0:D].T
        kb = k_rows(hr, hr)
        kmax = k_norm(jnp.concatenate([ka, kb], axis=0))
        qr = r1 // 4
        cp_wv.wait()
        x_copy(1).wait()
        for t in range(4):
            q_cols(t * qr, qr)
            if t == 0:
                wT_s[D:2 * D, :] = wqkv_ref[:, 2 * D:3 * D].T
            if t == 2:
                wT_s[2 * D:3 * D, :] = wqkv_ref[:, D:2 * D].T
            for z in range(qr // lp):
                ln_rows(r1 + t * qr + z * lp, lp)
        for i in range(2, n1):
            x_copy(i).wait()
        cp_mod2.start()
        cp_wo.start()
        cp_b1.start()
        cp_b2.start()
        cp_w1.start()
        cp_w2.start()
        for t in range(4):
            v_cols(t * qr, qr)
            for z in range(2 * qr // lp):
                ln_rows(2 * r1 + t * 2 * qr + z * lp, lp)

        def rows(i, kmax):
            rr = pl.multiple_of(i * r1, r1)
            kT = lax.dot_general(wT_s[2 * D:3 * D, :], h_s[pl.ds(rr, r1), :], NT, preferred_element_type=f32)
            k_s[pl.ds(rr, r1), :] = kT.astype(bf16).T
            kmax = jnp.maximum(kmax, jnp.sum((kT * kT).reshape(H, DH, r1), axis=1))
            q_cols(rr, r1)
            v_cols(rr, r1)
            return kmax
        kmax = lax.fori_loop(1, n1, rows, kmax)
        kn_s[...] = jnp.broadcast_to(jnp.sqrt(jnp.max(kmax, axis=1, keepdims=True)) * BOUND_SLACK, (H, 128))

        def pv_stage(s, d, cc):
            p = jnp.exp2(s.reshape(kc // 8, 8, bq) - d['m'][None])
            ls = jnp.sum(p, axis=0)
            d['l'] = ls if d['l'] is None else d['l'] + ls
            r = jnp.dot(vT_s[pl.ds(d['hoff'], DH), cc * kc:(cc + 1) * kc], p.reshape(kc, bq).astype(bf16),
                        preferred_element_type=f32)
            d['acc'] = r if d['acc'] is None else d['acc'] + r

        def finalize(d, safe):
            lsum = jnp.sum(d['l'], axis=0, keepdims=True)
            oT_s[pl.ds(d['hoff'], DH), pl.ds(d['q0'], bq)] = (d['acc'] * (1.0 / lsum)).astype(bf16)
            return jnp.where(lsum >= L_MIN, safe, 0.0)

        def prev_state(itp, l, acc, m):
            hp = (itp % G) * hu + (hu - 1)
            return dict(hoff=pl.multiple_of(hp * DH, DH), q0=pl.multiple_of((itp // G) * bq, bq), l=l, acc=acc, m=m)

        def heads(it, carry):
            safe, l_p, acc_p, m_p = carry
            prev = prev_state((it + nit - 1) % nit, l_p, acc_p, m_p)
            hg = it % G
            q0 = pl.multiple_of((it // G) * bq, bq)
            items = []
            st = {}
            for u in range(hu):
                h = hg * hu + u
                goff = pl.multiple_of((hg * hu + u) // 8 * 128, 128)
                hoff = pl.multiple_of(h * DH, DH)
                jj = u % 8
                parts = [qT_s[pl.ds(hoff, DH), pl.ds(q0, bq)]]
                if jj > 0:
                    parts.insert(0, jnp.zeros((DH * jj, bq), bf16))
                if jj < 7:
                    parts.append(jnp.zeros((DH * (7 - jj), bq), bf16))
                qm = jnp.concatenate(parts, axis=0)
                kn = jnp.concatenate([kn_s[pl.ds(h, 1), :]] * (bq // 128), axis=1)
                m = jnp.broadcast_to(qn_s[pl.ds(h, 1), pl.ds(q0, bq)] * kn, (8, bq))
                st[u] = dict(goff=goff, hoff=hoff, q0=q0, qm=qm, m=m, l=None, acc=None)
                for cc in range(nc):
                    items.append((u, cc))
            svals = {}
            n = len(items)
            for t in range(n):
                u, cc = items[t]
                d = st[u]
                svals[t] = jnp.dot(k_s[cc * kc:(cc + 1) * kc, pl.ds(d['goff'], 128)], d['qm'],
                                   preferred_element_type=f32)
                if t < lag:
                    pv_stage(sp_s[t], prev, nc - lag + t)
                    if t == lag - 1:
                        safe = finalize(prev, safe)
                else:
                    u, cc = items[t - lag]
                    pv_stage(svals.pop(t - lag), st[u], cc)
                    if cc == nc - 1:
                        safe = finalize(st[u], safe)
            for t in range(lag):
                sp_s[t] = svals.pop(n - lag + t)
            d = st[hu - 1]
            return safe, d['l'], d['acc'], d['m']

        sp_s[...] = jnp.zeros(sp_s.shape, f32)
        init = (jnp.full((1, bq), 1.0, f32), jnp.zeros((8, bq), f32), jnp.zeros((DH, bq), f32),
                jnp.zeros((8, bq), f32))
        safe, l_p, acc_p, m_p = lax.fori_loop(0, nit, heads, init)
        cp_mod2.wait()
        cp_wo.wait()
        cp_b1.wait()
        cp_b2.wait()
        cp_w1.wait()
        cp_w2.wait()

        def proj_ln(i, slot):
            rr = pl.multiple_of(i * r2, r2)
            attn = lax.dot_general(oT_s[:, pl.ds(rr, r2)], wo_ref[...], TN, preferred_element_type=f32)
            x1 = x_ref[pl.ds(rr, r2), :].astype(f32) + mod_s[0:1, 0:D] * attn
            x1_s[slot][...] = x1
            h = _ln(x1) * (1.0 + mod_s[0:1, 2 * D:3 * D]) + mod_s[0:1, D:2 * D]
            h2_s[slot][...] = h.astype(bf16)

        last = prev_state(nit - 1, l_p, acc_p, m_p)
        for t in range(lag):
            pv_stage(sp_s[t], last, nc - lag + t)
        safe = finalize(last, safe)
        mod_s[...] = jnp.dot(sc, wmod_ref[:, 2 * D:6 * D], preferred_element_type=f32)[0:8]
        proj_ln(0, 0)
        unsafe = jnp.min(safe) < 0.5

        @pl.when(unsafe)
        def _():
            row_f = lax.broadcasted_iota(jnp.int32, (128, 128), 0)

            def one(it, carry):
                h = it % H
                q0 = pl.multiple_of((it // H) * 128, 128)
                goff = pl.multiple_of(h // 8 * 128, 128)
                hoff = pl.multiple_of(h * DH, DH)
                qg = qT_s[pl.ds(goff, 128), pl.ds(q0, 128)]
                qm = jnp.where(row_f // DH == h % 8, qg, jnp.zeros_like(qg))
                s = jnp.dot(k_s[:, pl.ds(goff, 128)], qm, preferred_element_type=f32)
                p = jnp.exp2(s - jnp.max(s, axis=0, keepdims=True))
                l = jnp.sum(p, axis=0, keepdims=True)
                o = jnp.dot(vT_s[pl.ds(hoff, DH), :], p.astype(bf16), preferred_element_type=f32)
                oT_s[pl.ds(hoff, DH), pl.ds(q0, 128)] = (o / l).astype(bf16)
                return carry
            lax.fori_loop(0, (S // 128) * H, one, 0)
            proj_ln(0, 0)

        b1 = b1_ref[...].astype(f32).reshape(1, F)
        b2 = b2_ref[...].astype(f32).reshape(1, D)

        def out_copy(i):
            rr = pl.multiple_of(i * r2, r2)
            return pltpu.make_async_copy(out_s.at[pl.ds(rr, r2), :], o_hbm.at[pl.ds(rr, r2), :], osems.at[i])

        def ffn(i, slot, between):
            rr = pl.multiple_of(i * r2, r2)
            h1 = jnp.dot(h2_s[slot][...], w1_ref[...], preferred_element_type=f32) + b1
            h1 = jnp.maximum(h1, 0.0)
            h1 = (h1 * h1).astype(bf16)
            between()
            y = jnp.dot(h1, w2_ref[...], preferred_element_type=f32) + b2
            out_s[pl.ds(rr, r2), :] = (x1_s[slot][...] + mod_s[0:1, 3 * D:4 * D] * y).astype(out_s.dtype)
            out_copy(i).start()

        def tail(j, carry):
            i = 2 * j
            ffn(i, 0, lambda: proj_ln(i + 1, 1))
            ffn(i + 1, 1, lambda: proj_ln(jnp.minimum(i + 2, n2 - 1), 0))
            return carry
        lax.fori_loop(0, n2 // 2, tail, 0)
        for i in range(n2):
            out_copy(i).wait()

    any_spec = pl.BlockSpec(memory_space=pl.ANY)
    return functools.partial(
        pl.pallas_call,
        kernel,
        in_specs=[any_spec] * 9,
        out_specs=any_spec,
        scratch_shapes=[
            pltpu.VMEM((S, D), bf16), pltpu.VMEM((D, 3 * D), bf16), pltpu.VMEM((D, D), bf16),
            pltpu.VMEM((D, F), bf16), pltpu.VMEM((F, D), bf16), pltpu.VMEM((D, 6 * D), bf16),
            pltpu.VMEM((8, 4 * D), f32), pltpu.VMEM((3 * D, D), bf16), pltpu.VMEM((D, S), bf16),
            pltpu.VMEM((S, D), bf16), pltpu.VMEM((D, S), bf16), pltpu.VMEM((H, S), f32),
            pltpu.VMEM((H, 128), f32), pltpu.VMEM((D, S), bf16), pltpu.VMEM((S, D), bf16),
            pltpu.VMEM((S, D), bf16), pltpu.VMEM((lag, kc, bq), f32), pltpu.VMEM((r2, D), f32),
            pltpu.VMEM((r2, D), f32), pltpu.VMEM((r2, D), bf16), pltpu.VMEM((r2, D), bf16),
            pltpu.VMEM((1, D), bf16), pltpu.VMEM((F,), bf16), pltpu.VMEM((D,), bf16),
            pltpu.SemaphoreType.DMA((12,)), pltpu.SemaphoreType.DMA((n1,)), pltpu.SemaphoreType.DMA((n2,)),
        ],
        compiler_params=pltpu.CompilerParams(vmem_limit_bytes=100 * 1024 * 1024),
        name="fused_adaln_block",
    )


def _build(**kw):
    def fn(A_x, A_wqkv, A_wo, B_x, B_w1, B_b1, B_w2, B_b2, c, w_mod):
        del B_x
        out = make_kernel(**kw)(out_shape=jax.ShapeDtypeStruct((S, D), A_x.dtype))(
            A_x.reshape(S, D), A_wqkv, A_wo, B_w1, B_b1, B_w2, B_b2, c, w_mod)
        return out.reshape(A_x.shape)
    return fn


@jax.jit
def pallas_adaLN_cond__mha_block__dense_activation_squared_relu__prompt_kernel(
    A_x: jax.Array,
    A_wqkv: jax.Array,
    A_wo: jax.Array,
    B_x: jax.Array,
    B_w1: jax.Array,
    B_b1: jax.Array,
    B_w2: jax.Array,
    B_b2: jax.Array,
    c: jax.Array,
    w_mod: jax.Array,
):
    return _build()(A_x, A_wqkv, A_wo, B_x, B_w1, B_b1, B_w2, B_b2, c, w_mod)
```
